```python
import jax
import jax.numpy as jnp

def _softmax(x, axis=-1):
    return jax.nn.softmax(x, axis=axis)

def _gelu(x):
    return jax.nn.gelu(x, approximate=True)

def _silu(x):
    return jax.nn.silu(x)

def _sigmoid(x):
    return jax.nn.sigmoid(x)

def _layernorm(x, axis=-1, eps=1e-05):
    m = jnp.mean(x, axis=axis, keepdims=True)
    v = jnp.var(x, axis=axis, keepdims=True)
    return (x - m) / jnp.sqrt(v + eps)

def _scatter_add(tgt, idx, src, axis=0):
    return tgt.at[idx].add(src)

def _segment_sum(src, seg, n):
    return jax.ops.segment_sum(src, seg, n)

class _Rng:

    def __init__(self, key):
        self._k = key

    def _next(self):
        self._k, sub = jax.random.split(self._k)
        return sub

    def normal(self, shape):
        return jax.random.normal(self._next(), shape, dtype=jnp.bfloat16)

    def randint(self, lo, hi, shape):
        return jax.random.randint(self._next(), shape, lo, hi, dtype=jnp.int32)

    def uniform(self, shape, lo=0.0, hi=1.0):
        return jax.random.uniform(self._next(), shape, jnp.bfloat16, lo, hi)

    def permutation(self, n):
        return jax.random.permutation(self._next(), n)
kernel_name = 'concat_heads__spectral_gfnet__memory_aug_recurrent_mem_tr__prompt'

def setup_inputs():
    _rng = _Rng(jax.random.key(int.from_bytes(__import__("os").urandom(4), "little")))
    _w = lambda a: (lambda t: t.astype(jnp.bfloat16) if jnp.issubdtype(t.dtype, jnp.floating) else t)(jnp.asarray(a))

    def _A_setup():
        B, S, D = (1, 2048, 1024)
        Df = D // 2 + 1
        return {'x': _w((lambda *s: _rng.normal(s) * 0.05)(B, S, D)), 'w_r': _w((lambda *s: _rng.normal(s) * 0.05)(S, Df) * 0.02), 'w_i': _w((lambda *s: _rng.normal(s) * 0.05)(S, Df) * 0.02)}
    _A_in = _A_setup()

    def _B_setup():
        B, S, Dm = (1, 2048, 1024)
        H, Dh = (32, 128)
        M, seg = (8, 32)
        seg = min(seg, S)
        S = S // seg * seg
        return {'x': _w((lambda *s: _rng.normal(s) * 0.05)(B, S, Dm)), 'mem0': _w((lambda *s: _rng.normal(s) * 0.05)(B, M, Dm)), 'Wq': _w((lambda *s: _rng.normal(s) * 0.05)(Dm, H, Dh) * Dm ** (-0.5)), 'Wk': _w((lambda *s: _rng.normal(s) * 0.05)(Dm, H, Dh) * Dm ** (-0.5)), 'Wv': _w((lambda *s: _rng.normal(s) * 0.05)(Dm, H, Dh) * Dm ** (-0.5)), 'Wo': _w((lambda *s: _rng.normal(s) * 0.05)(H, Dh, Dm) * (H * Dh) ** (-0.5)), 'seg_len': seg}
    _B_in = _B_setup()
    return {'A_x': _A_in['x'], 'A_w_r': _A_in['w_r'], 'A_w_i': _A_in['w_i'], 'B_x': _B_in['x'], 'B_mem0': _B_in['mem0'], 'B_Wq': _B_in['Wq'], 'B_Wk': _B_in['Wk'], 'B_Wv': _B_in['Wv'], 'B_Wo': _B_in['Wo'], 'B_seg_len': _B_in['seg_len']}

def reference(A_x, A_w_r, A_w_i, B_x, B_mem0, B_Wq, B_Wk, B_Wv, B_Wo, B_seg_len):

    def _A_ref(x, w_r, w_i):
        B, S, D = x.shape
        X = (lambda x, axes=(-2, -1): jnp.fft.rfft2(x.astype(jnp.float32), axes=axes))(x, axes=(-2, -1))
        W = w_r + 1j * w_i
        X = X * W
        y = (lambda x, s, axes=(-2, -1): jnp.fft.irfft2(x, s=s, axes=axes).astype(jnp.bfloat16))(X, (S, D), axes=(-2, -1))
        return y

    def _B_ref(x, mem0, Wq, Wk, Wv, Wo, seg_len):
        B, S, Dm = x.shape
        H, Dh = (Wq.shape[1], Wq.shape[2])
        M = mem0.shape[1]
        scale = Dh ** (-0.5)
        n_seg = S // seg_len
        L = M + seg_len
        idx = jnp.arange(L)
        mask = (idx[:, None] < M) | (idx[:, None] >= idx[None, :])
        mem = mem0
        outs = []
        for s in range(n_seg):
            xs = x[:, s * seg_len:(s + 1) * seg_len, :].copy()
            h = jnp.concatenate([mem, xs], axis=1)
            q = jnp.einsum('btd,dhe->bhte', h, Wq)
            k = jnp.einsum('btd,dhe->bhte', h, Wk)
            v = jnp.einsum('btd,dhe->bhte', h, Wv)
            scores = jnp.einsum('bhqe,bhke->bhqk', q, k) * scale
            scores = jnp.where(mask[None, None], scores, -1000000000.0)
            p = _softmax(scores, axis=-1)
            o = jnp.einsum('bhqk,bhke->bhqe', p, v)
            o = jnp.einsum('bhte,hed->btd', o, Wo)
            mem = o[:, :M, :].copy()
            outs.append(o[:, M:, :])
        return jnp.concatenate(outs, axis=1)
    a = _A_ref(A_x, A_w_r, A_w_i)
    b = _B_ref(B_x, B_mem0, B_Wq, B_Wk, B_Wv, B_Wo, B_seg_len)
    return jnp.concatenate([a, b], axis=-1)
```

```python
import functools

import jax
import jax.numpy as jnp
import ml_dtypes
import numpy as np
from jax import lax
import jax.experimental.pallas as pl
import jax.experimental.pallas.tpu as pltpu

S_, D_, H_, DH_, M_, SEG_ = 2048, 1024, 32, 128, 8, 32
L_ = M_ + SEG_
NSEG_ = S_ // SEG_
KR_ = 520
f32, bf16, u32 = jnp.float32, jnp.bfloat16, jnp.uint32
HI16 = np.uint32(0xFFFF0000)
LO16 = np.uint32(0xFFFF)
R2 = float(np.sqrt(0.5))


def _dft_constants():
    th = 2 * np.pi / D_
    b = np.arange(128)
    j = np.arange(64)

    def cs(k):
        ang = th * ((k[:, None] * b[None, :]) % D_)
        return np.cos(ang), np.sin(ang)

    c0, s0 = cs(8 * j)
    c4, s4 = cs(4 + 8 * j)
    alt = (-1.0) ** b
    nyq = np.zeros((16, 128))
    nyq[0] = alt
    l0 = np.concatenate([c0, -s0], 0)
    l4 = np.concatenate([c4, -s4], 0)
    i0 = l0.copy()
    i0[0] *= 0.5
    i0[64] = 0.5 * alt
    mats = [l0, l4, i0]
    for r in (1, 2, 3):
        ca, sa = cs(r + 8 * j)
        cb, sb = cs(8 - r + 8 * j)
        mats += [np.concatenate([ca, cb], 0), np.concatenate([-sa, sb], 0)]
    dmat = np.concatenate(mats + [nyq], 0)
    n1 = np.arange(128)
    ms = []
    for n2 in range(16):
        ang = 2 * np.pi / S_ * (((16 * n1 + n2)[:, None] * n1[None, :]) % S_)
        ms.append(np.stack([np.cos(ang), -np.sin(ang)]) * 2.0 ** -10)
    return dmat.astype(ml_dtypes.bfloat16), np.stack(ms).astype(ml_dtypes.bfloat16)


_DMAT, _SMAT = _dft_constants()


def _dot_nt(a, b):
    return lax.dot_general(a, b, (((1,), (1,)), ((), ())), preferred_element_type=f32)


def _dot(a, b):
    return jnp.dot(a, b, preferred_element_type=f32)


def _radix4(xs, sgn):
    (ar, ai), (br, bi), (cr, ci), (dr, di) = xs
    t0r, t0i = ar + cr, ai + ci
    t1r, t1i = ar - cr, ai - ci
    t2r, t2i = br + dr, bi + di
    t3r, t3i = br - dr, bi - di
    y0 = (t0r + t2r, t0i + t2i)
    y2 = (t0r - t2r, t0i - t2i)
    ym = (t1r + t3i, t1i - t3r)
    yp = (t1r - t3i, t1i + t3r)
    return [y0, ym, y2, yp] if sgn < 0 else [y0, yp, y2, ym]


def _twiddle16(z, e, sgn):
    r, i = z
    if e == 0:
        return z
    if e == 4:
        return (-i, r) if sgn > 0 else (i, -r)
    if e == 2:
        return ((r - i) * R2, (r + i) * R2) if sgn > 0 else ((r + i) * R2, (i - r) * R2)
    if e == 6:
        return ((-r - i) * R2, (r - i) * R2) if sgn > 0 else ((i - r) * R2, (-r - i) * R2)
    c = float(np.cos(2 * np.pi * e / 16))
    s = float(sgn * np.sin(2 * np.pi * e / 16))
    return (r * c - i * s, r * s + i * c)


def _fft16(xs, sgn):
    a = [_radix4([xs[4 * p + q] for p in range(4)], sgn) for q in range(4)]
    out = [None] * 16
    for u in range(4):
        y = _radix4([_twiddle16(a[q][u], q * u, sgn) for q in range(4)], sgn)
        for v in range(4):
            out[u + 4 * v] = y[v]
    return out


def _segment_schedule(lag_s=2, lag_p=2, group=4, hold=2):
    ng = H_ // group
    tail = {H_ + i * (lag_s + lag_p) // hold: g for i, g in enumerate(range(ng - 1 - hold, ng - 1))}
    sched = []
    for i in range(H_ + lag_s + lag_p):
        if i < H_:
            sched.append(("qkv", i))
        if i in tail:
            sched.append(("o", tail[i] * group, (tail[i] + 1) * group))
        if 0 <= i - lag_s < H_:
            sched.append(("s", i - lag_s))
        if 0 <= i - lag_s - lag_p < H_:
            sched.append(("pv", i - lag_s - lag_p))
        hp = i - lag_s - lag_p - 1
        if hp >= 0 and hp % group == group - 1 and hp // group < ng - 1 - hold:
            sched.append(("o", hp + 1 - group, hp + 1))
    sched.append(("o", (ng - 1) * group, H_))
    return sched


def _kernel(ax_hbm, wrt_hbm, wit_hbm, wrn_ref, win_ref, dmat_hbm, smat_hbm,
            bx_hbm, m0_ref, wq_hbm, wk_hbm, wv_hbm, wo_hbm, out_hbm,
            xg_ref, y_ref, t_ref, fw_ref, dmat_ref, smat_ref,
            w_ref, wo_ref, bx_ref, outb_ref,
            sem_ax, sem_fw, sem_c, sem_w, sem_wo, sem_bx, sem_outa, sem_outb):
    unroll = 2

    axu = ax_hbm.bitcast(u32)

    def ax_copy(c):
        return pltpu.make_async_copy(axu.at[:, c], xg_ref.at[c], sem_ax.at[c])

    cd = pltpu.make_async_copy(dmat_hbm, dmat_ref, sem_c.at[0])
    cs = pltpu.make_async_copy(smat_hbm, smat_ref, sem_c.at[1])
    cd.start()
    ax_copy(0).start()
    cs.start()
    for c in range(1, 8):
        ax_copy(c).start()
    fw_copies = []
    for ri, wh in enumerate((wrt_hbm, wit_hbm)):
        wu = wh.at[pl.ds(0, 512)].bitcast(u32)
        for k2 in range(16):
            cp = pltpu.make_async_copy(wu.at[:, pl.ds(k2 * 128, 128)], fw_ref.at[ri, k2], sem_fw.at[0])
            cp.start()
            fw_copies.append(cp)
    w_copies = []
    for mi, whbm in enumerate((wq_hbm, wk_hbm, wv_hbm)):
        wu = whbm.bitcast(u32)
        for j in range(16):
            for par in range(2):
                cp = pltpu.make_async_copy(wu.at[:, par * 16 + j], w_ref.at[mi, 2 * j + par], sem_w.at[0])
                cp.start()
                w_copies.append(cp)
    wou = wo_hbm.bitcast(u32)
    wo_copies = []
    for n in range(8):
        cp = pltpu.make_async_copy(wou.at[:, pl.ds(n * 128, 128)], wo_ref.at[n], sem_wo.at[0])
        cp.start()
        wo_copies.append(cp)
    bx_copy = pltpu.make_async_copy(bx_hbm, bx_ref, sem_bx.at[0])
    bx_copy.start()
    cd.wait()
    cs.wait()

    def dm(i):
        return dmat_ref[i * 128:(i + 1) * 128, :]

    def fwd(c, carry):
        ax_copy(c).wait()
        for r0 in range(0, 128, 16):
            w = [xg_ref[c, r0:r0 + 16, a * 128:(a + 1) * 128] for a in range(8)]
            for par in range(2):
                xa = [pltpu.bitcast((v << 16) if par == 0 else (v & HI16), f32) for v in w]
                t0, t1 = xa[0] + xa[4], xa[0] - xa[4]
                t2, t3 = xa[2] + xa[6], xa[2] - xa[6]
                t4, t5 = xa[1] + xa[5], xa[1] - xa[5]
                t6, t7 = xa[3] + xa[7], xa[3] - xa[7]
                e, o = t0 + t2, t4 + t6
                u, v = (t5 - t7) * R2, (t5 + t7) * R2
                ys = [e + o, e - o, t1 + u, -t3 - v, t0 - t2, t6 - t4, t1 - u, t3 - v]
                for i, yv in enumerate(ys):
                    y_ref[par, i, r0:r0 + 16, :] = yv.astype(bf16)
        for par in range(2):
            n2 = 2 * c + par
            z0 = _dot_nt(dm(0), y_ref[par, 0])
            zn = _dot_nt(dmat_ref[9 * 128:9 * 128 + 16, :], y_ref[par, 0])
            z4 = _dot_nt(dm(1), y_ref[par, 1])
            zr = [z0[0:64], z4[0:64]]
            zi = [z0[64:128], z4[64:128]]
            for r in range(3):
                cd_ = jnp.concatenate([dm(3 + 2 * r), dm(4 + 2 * r)], axis=0)
                a = _dot_nt(cd_, y_ref[par, 2 + 2 * r])
                b = _dot_nt(cd_, y_ref[par, 3 + 2 * r])
                zr.append(a[0:128] - b[128:256])
                zi += [a[128:192] + b[0:64], -a[192:256] - b[64:128]]
            zr.append(zn)
            zi.append(jnp.zeros((16, 128), f32))
            zr = jnp.concatenate(zr, axis=0).astype(bf16)
            zi = jnp.concatenate(zi, axis=0).astype(bf16)
            mcd = jnp.concatenate([smat_ref[n2, 0], smat_ref[n2, 1]], axis=1)
            a = _dot(zr, mcd)
            b = _dot(zi, mcd)
            t_ref[0, n2] = (a[:, 0:128] - b[:, 128:256])[0:KR_]
            t_ref[1, n2] = (a[:, 128:256] + b[:, 0:128])[0:KR_]
        return carry

    lax.fori_loop(0, 8, fwd, 0)

    for cp in fw_copies:
        cp.wait()

    def mid_group(row0, getw):
        xs = [(t_ref[0, n2, pl.ds(row0, 8), :], t_ref[1, n2, pl.ds(row0, 8), :]) for n2 in range(16)]
        xf = _fft16(xs, -1)
        prod = []
        for k2 in range(16):
            wr, wi = getw(k2)
            xr, xi = xf[k2]
            prod.append((xr * wr - xi * wi, xr * wi + xi * wr))
        vs = _fft16(prod, +1)
        for n2 in range(16):
            t_ref[0, n2, pl.ds(row0, 8), :] = vs[n2][0]
            t_ref[1, n2, pl.ds(row0, 8), :] = vs[n2][1]

    for blk, r in enumerate((0, 4, 1, 7, 2, 6, 3, 5)):
        def mid(g, carry, blk=blk, r=r):
            def getw(k2):
                idx = pl.ds(g * 32 + r // 2, 8, stride=4)
                a = fw_ref[0, k2, idx, :]
                b = fw_ref[1, k2, idx, :]
                if r % 2 == 0:
                    a, b = a << 16, b << 16
                else:
                    a, b = a & HI16, b & HI16
                return pltpu.bitcast(a, f32), pltpu.bitcast(b, f32)

            mid_group(pl.multiple_of(blk * 64 + g * 8, 8), getw)
            return carry

        lax.fori_loop(0, 8, mid, 0)

    def getw_nyquist(k2):
        a = wrn_ref[0:1, k2 * 128:(k2 + 1) * 128].astype(f32)
        b = win_ref[0:1, k2 * 128:(k2 + 1) * 128].astype(f32)
        return jnp.broadcast_to(a, (8, 128)), jnp.broadcast_to(b, (8, 128))

    mid_group(512, getw_nyquist)

    outu = out_hbm.bitcast(u32)

    def outa_copy(c):
        return pltpu.make_async_copy(xg_ref.at[c], outu.at[:, c, pl.ds(0, D_)], sem_outa.at[0])

    def inv(c, carry):
        row = lax.broadcasted_iota(jnp.int32, (8, 128), 0)
        lane = lax.broadcasted_iota(jnp.int32, (1, 128), 1)
        sgn = jnp.where(lane < 64, 1.0, -1.0).astype(f32)
        res = []
        for par in range(2):
            n2 = 2 * c + par
            mc = smat_ref[n2, 0]
            md = smat_ref[n2, 1]
            mcd = jnp.concatenate([mc, md], axis=1)
            vr, vi = t_ref[0, n2, 0:64, :], t_ref[1, n2, 0:64, :]
            nr, ni = t_ref[0, n2, 512:520, :], t_ref[1, n2, 512:520, :]
            vi0 = jnp.concatenate([jnp.where(row == 0, nr, vi[0:8]), vi[8:64]], axis=0)
            vr0 = jnp.concatenate([jnp.where(row == 0, ni, -vr[0:8]), -vr[8:64]], axis=0)
            ra = jnp.concatenate([jnp.concatenate([vr, vi0], axis=0),
                                  jnp.concatenate([vi, vr0], axis=0)], axis=1).astype(bf16)
            ta = _dot_nt(mcd, ra)
            vr, vi = t_ref[0, n2, 64:128, :], t_ref[1, n2, 64:128, :]
            rb = jnp.concatenate([jnp.concatenate([vr, vi], axis=0),
                                  jnp.concatenate([vi, -vr], axis=0)], axis=1).astype(bf16)
            tb = _dot_nt(mcd, rb)
            g0 = _dot(ta, dm(2))
            g4 = _dot(tb, dm(1))
            mcd2 = jnp.concatenate([mc, md], axis=0)
            hr, hi = [], []
            for r in range(3):
                vr = t_ref[0, n2, 128 * (r + 1):128 * (r + 2), :].astype(bf16)
                vi = t_ref[1, n2, 128 * (r + 1):128 * (r + 2), :].astype(bf16)
                a = _dot_nt(mcd2, vr)
                b = _dot_nt(mcd2, vi)
                ur = a[0:128] + b[128:256]
                ui = (b[0:128] - a[128:256]) * sgn
                cd_ = jnp.concatenate([dm(3 + 2 * r), dm(4 + 2 * r)], axis=1)
                a = _dot(ur, cd_)
                b = _dot(ui, cd_)
                hr.append(a[:, 0:128] + b[:, 128:256])
                hi.append(b[:, 0:128] - a[:, 128:256])
            ep, em = g0 + g4, g0 - g4
            s13 = hr[0] + hr[2]
            d13 = hi[0] - hi[2]
            p = ((hr[0] - hi[0]) - (hr[2] + hi[2])) * R2
            q = ((hr[2] - hi[2]) - (hr[0] + hi[0])) * R2
            e1, e2 = ep + hr[1], ep - hr[1]
            e3, e4 = em - hi[1], em + hi[1]
            res.append([e1 + s13, e3 + p, e2 - d13, e4 + q, e1 - s13, e3 - p, e2 + d13, e4 - q])
        for a in range(8):
            wv = pltpu.pack_elementwise([res[0][a], res[1][a]], packed_dtype=bf16)
            xg_ref[c, :, a * 128:(a + 1) * 128] = pltpu.bitcast(wv, u32)
        outa_copy(c).start()
        return carry

    lax.fori_loop(0, 8, inv, 0)

    for cp in w_copies:
        cp.wait()

    def relayout(i, carry):
        mi = i // 16
        j = i % 16
        for r in range(0, 512, 128):
            a = w_ref[mi, 2 * j, r:r + 128, :]
            b = w_ref[mi, 2 * j + 1, r:r + 128, :]
            w_ref[mi, 2 * j, r:r + 128, :] = (a & LO16) | (b << 16)
            w_ref[mi, 2 * j + 1, r:r + 128, :] = (a >> 16) | (b & HI16)
        return carry

    lax.fori_loop(0, 48, relayout, 0)
    for cp in wo_copies:
        cp.wait()
    bx_copy.wait()

    scale = DH_ ** -0.5
    sched = _segment_schedule()

    def segment(s, mem):
        r0 = pl.multiple_of(s * SEG_, SEG_)
        row = lax.broadcasted_iota(jnp.int32, (L_, L_), 0)
        col = lax.broadcasted_iota(jnp.int32, (L_, L_), 1)
        mask = (row < M_) | (row >= col)
        xs = bx_ref[pl.ds(r0, SEG_), :].astype(f32)
        hh = jnp.concatenate(
            [jnp.concatenate([mem[n], xs[:, n * 128:(n + 1) * 128]], axis=0) for n in range(8)], axis=1)
        qkv, probs, att = {}, {}, {}
        acc = [None] * 8
        for op in sched:
            if op[0] == "qkv":
                h = op[1]
                q, k, v = [_dot(hh, pltpu.bitcast(w_ref[mi, h], bf16)) for mi in range(3)]
                qkv[h] = (q, k.astype(bf16), v.astype(bf16))
            elif op[0] == "s":
                q, k, v = qkv.pop(op[1])
                sc = jnp.where(mask, _dot_nt(q, k) * scale, -1e9)
                e = jnp.exp(sc - jnp.max(sc, axis=-1, keepdims=True))
                probs[op[1]] = (e, v, 1.0 / jnp.sum(e, axis=-1, keepdims=True))
            elif op[0] == "pv":
                e, v, rl = probs.pop(op[1])
                att[op[1]] = _dot(e, v) * rl
            else:
                _, h0, h1 = op
                og = jnp.concatenate([att.pop(h) for h in range(h0, h1)], axis=1)
                for n in range(8):
                    y = _dot(og, pltpu.bitcast(wo_ref[n, h0 * 64:h1 * 64, :], bf16))
                    acc[n] = y if acc[n] is None else acc[n] + y
        for n in range(8):
            yb = acc[n][M_:L_].astype(bf16)
            outb_ref[2 * s, :, n * 128:(n + 1) * 128] = yb[0:16]
            outb_ref[2 * s + 1, :, n * 128:(n + 1) * 128] = yb[16:32]
        return [acc[n][0:M_] for n in range(8)]

    def body(i, mem):
        mem = list(mem)
        for u in range(unroll):
            mem = segment(i * unroll + u, mem)
        blk = pl.ds(i * (2 * unroll), 2 * unroll)
        pltpu.make_async_copy(outb_ref.at[blk], out_hbm.at[blk, :, pl.ds(D_, D_)], sem_outb.at[0]).start()
        return tuple(mem)

    m0 = m0_ref[...].astype(f32)
    lax.fori_loop(0, NSEG_ // unroll, body, tuple(m0[:, n * 128:(n + 1) * 128] for n in range(8)))
    for c in range(8):
        outa_copy(c).wait()
    pltpu.make_async_copy(outb_ref, out_hbm.at[:, :, pl.ds(D_, D_)], sem_outb.at[0]).wait()


@functools.partial(jax.jit, static_argnames=("B_seg_len",))
def pallas_concat_heads__spectral_gfnet__memory_aug_recurrent_mem_tr__prompt_kernel(
    A_x: jax.Array,
    A_w_r: jax.Array,
    A_w_i: jax.Array,
    B_x: jax.Array,
    B_mem0: jax.Array,
    B_Wq: jax.Array,
    B_Wk: jax.Array,
    B_Wv: jax.Array,
    B_Wo: jax.Array,
    B_seg_len: int,
):
    assert B_seg_len == SEG_
    assert A_x.shape == (1, S_, D_) and B_x.shape == (1, S_, D_)
    assert B_Wq.shape == (D_, H_, DH_) and B_mem0.shape == (1, M_, D_)
    wrt, wit = A_w_r.T, A_w_i.T
    hbm = pl.BlockSpec(memory_space=pltpu.HBM)
    nyq = pl.BlockSpec((8, S_), lambda i: (64, 0))
    dma = pltpu.SemaphoreType.DMA
    out = pl.pallas_call(
        _kernel,
        grid=(1,),
        out_shape=jax.ShapeDtypeStruct((128, 16, 2 * D_), bf16),
        in_specs=[hbm, hbm, hbm, nyq, nyq, hbm, hbm,
                  hbm, pl.BlockSpec((M_, D_), lambda i: (0, 0)), hbm, hbm, hbm, hbm],
        out_specs=hbm,
        scratch_shapes=[
            pltpu.VMEM((8, 128, D_), u32),
            pltpu.VMEM((2, 8, 128, 128), bf16),
            pltpu.VMEM((2, 16, KR_, 128), f32),
            pltpu.VMEM((2, 16, 256, 128), u32),
            pltpu.VMEM(_DMAT.shape, bf16),
            pltpu.VMEM(_SMAT.shape, bf16),
            pltpu.VMEM((3, H_, 512, 128), u32),
            pltpu.VMEM((8, 2048, 128), u32),
            pltpu.VMEM((S_, D_), bf16),
            pltpu.VMEM((128, 16, D_), bf16),
            dma((8,)), dma((1,)), dma((2,)), dma((1,)), dma((1,)), dma((1,)), dma((1,)), dma((1,)),
        ],
        compiler_params=pltpu.CompilerParams(
            dimension_semantics=("arbitrary",), vmem_limit_bytes=110 * 1024 * 1024),
    )(A_x.reshape(128, 16, D_), wrt, wit, wrt, wit, _DMAT, _SMAT,
      B_x.reshape(S_, D_), B_mem0.reshape(M_, D_),
      B_Wq.reshape(512, 64, DH_), B_Wk.reshape(512, 64, DH_), B_Wv.reshape(512, 64, DH_),
      B_Wo.reshape(H_ * DH_, D_))
    return out.reshape(1, S_, 2 * D_)
```

```python
import functools

import jax
import jax.numpy as jnp
import ml_dtypes
import numpy as np
from jax import lax
import jax.experimental.pallas as pl
import jax.experimental.pallas.tpu as pltpu

S_, D_, H_, DH_, M_, SEG_ = 2048, 1024, 32, 128, 8, 32
L_ = M_ + SEG_
NSEG_ = S_ // SEG_
PRE_ = 8
TOK_ = SEG_ - PRE_
KR_ = 520
AHEAD_ = 3
f32, bf16, u32 = jnp.float32, jnp.bfloat16, jnp.uint32
HI16 = np.uint32(0xFFFF0000)
LO16 = np.uint32(0xFFFF)
R2 = float(np.sqrt(0.5))
LOG2E = float(np.log2(np.e))


def _dft_constants():
    th = 2 * np.pi / D_
    b = np.arange(128)
    j = np.arange(64)

    def cs(k):
        ang = th * ((k[:, None] * b[None, :]) % D_)
        return np.cos(ang), np.sin(ang)

    c0, s0 = cs(8 * j)
    c4, s4 = cs(4 + 8 * j)
    alt = (-1.0) ** b
    nyq = np.zeros((16, 128))
    nyq[0] = alt
    l0 = np.concatenate([c0, -s0], 0)
    l4 = np.concatenate([c4, -s4], 0)
    i0 = l0.copy()
    i0[0] *= 0.5
    i0[64] = 0.5 * alt
    mats = [l4, i0]
    lower = np.where(np.arange(128) < 64, 1.0, -1.0)[:, None]
    for r in (1, 2, 3):
        ca, sa = cs(r + 8 * j)
        cb, sb = cs(8 - r + 8 * j)
        c = np.concatenate([ca, cb], 0)
        d = np.concatenate([-sa, sb], 0)
        mats += [c, d - c, c + d, (d - c) * lower]
    dmat = np.concatenate(mats + [l0, nyq], 0)
    n1 = np.arange(128)
    ms = []
    for n2 in range(16):
        ang = 2 * np.pi / S_ * (((16 * n1 + n2)[:, None] * n1[None, :]) % S_)
        c, d = np.cos(ang), -np.sin(ang)
        ms.append(np.stack([c, d, d - c, c + d]) * 2.0 ** -10)

    def words(m):
        u = m.astype(ml_dtypes.bfloat16).view(np.uint16).astype(np.uint32)
        return u[..., 0::2, :] | (u[..., 1::2, :] << 16)

    return words(dmat), words(np.stack(ms))


_DMAT, _SMAT = _dft_constants()


def _bf(words):
    return pltpu.bitcast(words, bf16)


def _dot_nt(a, b):
    return lax.dot_general(a, b, (((1,), (1,)), ((), ())), preferred_element_type=f32)


def _dot(a, b):
    return jnp.dot(a, b, preferred_element_type=f32)


def _radix4(xs, sgn):
    (ar, ai), (br, bi), (cr, ci), (dr, di) = xs
    t0r, t0i = ar + cr, ai + ci
    t1r, t1i = ar - cr, ai - ci
    t2r, t2i = br + dr, bi + di
    t3r, t3i = br - dr, bi - di
    y0 = (t0r + t2r, t0i + t2i)
    y2 = (t0r - t2r, t0i - t2i)
    ym = (t1r + t3i, t1i - t3r)
    yp = (t1r - t3i, t1i + t3r)
    return [y0, ym, y2, yp] if sgn < 0 else [y0, yp, y2, ym]


def _twiddle16(z, e, sgn):
    r, i = z
    if e == 0:
        return z
    if e == 4:
        return (-i, r) if sgn > 0 else (i, -r)
    if e == 2:
        return ((r - i) * R2, (r + i) * R2) if sgn > 0 else ((r + i) * R2, (i - r) * R2)
    if e == 6:
        return ((-r - i) * R2, (r - i) * R2) if sgn > 0 else ((i - r) * R2, (-r - i) * R2)
    c = float(np.cos(2 * np.pi * e / 16))
    s = float(sgn * np.sin(2 * np.pi * e / 16))
    return (r * c - i * s, r * s + i * c)


def _fft16(xs, sgn):
    a = [_radix4([xs[4 * p + q] for p in range(4)], sgn) for q in range(4)]
    out = [None] * 16
    for u in range(4):
        y = _radix4([_twiddle16(a[q][u], q * u, sgn) for q in range(4)], sgn)
        for v in range(4):
            out[u + 4 * v] = y[v]
    return out


def _feature_butterflies(xg_ref, y_ref, c, slot):
    for r0 in range(0, 128, 16):
        w = [xg_ref[c, r0:r0 + 16, a * 128:(a + 1) * 128] for a in range(8)]
        for par in range(2):
            xa = [pltpu.bitcast((v << 16) if par == 0 else (v & HI16), f32) for v in w]
            t0, t1 = xa[0] + xa[4], xa[0] - xa[4]
            t2, t3 = xa[2] + xa[6], xa[2] - xa[6]
            t4, t5 = xa[1] + xa[5], xa[1] - xa[5]
            t6, t7 = xa[3] + xa[7], xa[3] - xa[7]
            e, o = t0 + t2, t4 + t6
            u, v = (t5 - t7) * R2, (t5 + t7) * R2
            p1, q1 = t1 + u, -t3 - v
            p2, q2 = t0 - t2, t6 - t4
            p3, q3 = t1 - u, t3 - v
            ys = [e + o, e - o, p1, q1, p1 + q1, p2, q2, p2 + q2, p3, q3, p3 + q3]
            for i, yv in enumerate(ys):
                y_ref[slot, par, i, r0 // 2:r0 // 2 + 8, :] = pltpu.bitcast(yv.astype(bf16), u32)


def _forward_matmuls(y_ref, t_ref, dmat_ref, smat_ref, n2, slot, par):
    def dm(i):
        return _bf(dmat_ref[i * 64:(i + 1) * 64, :])

    def y(i):
        return _bf(y_ref[slot, par, i])

    def feature_stage(r):
        if r == 0:
            z0 = _dot_nt(_bf(dmat_ref[14 * 64:14 * 64 + 72, :]), y(0))
            z4 = _dot_nt(dm(0), y(1))
            return (jnp.concatenate([z0[0:64], z4[0:64]], axis=0),
                    jnp.concatenate([z0[64:128], z4[64:128]], axis=0), z0[128:144])
        k1 = _dot_nt(dm(4 * r - 2), y(3 * r + 1))
        k2 = _dot_nt(dm(4 * r + 1), y(3 * r - 1))
        k3 = _dot_nt(dm(4 * r), y(3 * r))
        return k1 - k3, jnp.concatenate([k1[0:64] + k2[0:64], k2[64:128] - k1[64:128]], axis=0), None

    def sequence_stage(r, zr, zi, zn):
        zs = zr + zi
        if zn is not None:
            zs, zr = jnp.concatenate([zs, zn], axis=0), jnp.concatenate([zr, zn], axis=0)
        k1 = _dot(zs.astype(bf16), _bf(smat_ref[n2, 0]))
        k2 = _dot(zr.astype(bf16), _bf(smat_ref[n2, 2]))
        k3 = _dot(zi.astype(bf16), _bf(smat_ref[n2, 3]))
        re, im = k1[0:128] - k3, k1 + k2
        ra, rb = (0, 4) if r == 0 else (r, 8 - r)
        for ri, v in enumerate((re, im)):
            t_ref[ri, n2, 64 * ra:64 * ra + 64, :] = v[0:64]
            t_ref[ri, n2, 64 * rb:64 * rb + 64, :] = v[64:128]
        if zn is not None:
            t_ref[0, n2, 512:KR_, :] = k1[128:136]
            t_ref[1, n2, 512:KR_, :] = im[128:136]

    z = feature_stage(0)
    for r in range(4):
        z_next = feature_stage(r + 1) if r < 3 else None
        sequence_stage(r, *z)
        z = z_next


def _inverse_matmuls(t_ref, dmat_ref, smat_ref, n2):
    def dm(i):
        return _bf(dmat_ref[i * 64:(i + 1) * 64, :])

    row = lax.broadcasted_iota(jnp.int32, (8, 128), 0)
    lane = lax.broadcasted_iota(jnp.int32, (1, 128), 1)
    sgn = jnp.where(lane < 64, 1.0, -1.0).astype(f32)
    mcd = jnp.concatenate([_bf(smat_ref[n2, 0]), _bf(smat_ref[n2, 1])], axis=1)
    vr, vi = t_ref[0, n2, 0:64, :], t_ref[1, n2, 0:64, :]
    nr, ni = t_ref[0, n2, 512:KR_, :], t_ref[1, n2, 512:KR_, :]
    vi0 = jnp.concatenate([jnp.where(row == 0, nr, vi[0:8]), vi[8:64]], axis=0)
    vr0 = jnp.concatenate([jnp.where(row == 0, ni, -vr[0:8]), -vr[8:64]], axis=0)
    ra = jnp.concatenate([jnp.concatenate([vr, vi0], axis=0),
                          jnp.concatenate([vi, vr0], axis=0)], axis=1).astype(bf16)
    ta = _dot_nt(mcd, ra)
    vr, vi = t_ref[0, n2, 256:320, :], t_ref[1, n2, 256:320, :]
    rb = jnp.concatenate([jnp.concatenate([vr, vi], axis=0),
                          jnp.concatenate([vi, -vr], axis=0)], axis=1).astype(bf16)
    tb = _dot_nt(mcd, rb)
    us = []
    for r in (1, 2, 3):
        vr, vi = [jnp.concatenate([t_ref[ri, n2, 64 * r:64 * r + 64, :],
                                   t_ref[ri, n2, 64 * (8 - r):64 * (9 - r), :]], axis=0) for ri in range(2)]
        k1 = _dot_nt(_bf(smat_ref[n2, 0]), (vr + vi).astype(bf16))
        k2 = _dot_nt(_bf(smat_ref[n2, 3]), vr.astype(bf16))
        k3 = _dot_nt(_bf(smat_ref[n2, 2]), vi.astype(bf16))
        us.append((k1 + k3, (k1 - k2) * sgn))
    g0 = _dot(ta, dm(1))
    g4 = _dot(tb, dm(0))
    hr, hi = [], []
    for r in (1, 2, 3):
        ur, ui = us[r - 1]
        k1 = _dot(ur + ui, dm(4 * r - 2))
        k2 = _dot(ur, dm(4 * r))
        k3 = _dot(ui, dm(4 * r - 1))
        hr.append(k1 + k3)
        hi.append(k1 - k2)
    ep, em = g0 + g4, g0 - g4
    s13 = hr[0] + hr[2]
    d13 = hi[0] - hi[2]
    p = ((hr[0] - hi[0]) - (hr[2] + hi[2])) * R2
    q = ((hr[2] - hi[2]) - (hr[0] + hi[0])) * R2
    e1, e2 = ep + hr[1], ep - hr[1]
    e3, e4 = em - hi[1], em + hi[1]
    return [e1 + s13, e3 + p, e2 - d13, e4 + q, e1 - s13, e3 - p, e2 + d13, e4 - q]


def _filter_rows(t_ref, row0, get_w):
    rows = pl.ds(row0, 8)
    xf = _fft16([(t_ref[0, n2, rows, :], t_ref[1, n2, rows, :]) for n2 in range(16)], -1)
    prod = []
    for k2 in range(16):
        wr, wi = get_w(k2)
        xr, xi = xf[k2]
        prod.append((xr * wr - xi * wi, xr * wi + xi * wr))
    vs = _fft16(prod, +1)
    for n2 in range(16):
        t_ref[0, n2, rows, :] = vs[n2][0]
        t_ref[1, n2, rows, :] = vs[n2][1]


def _segment_schedule(order="s2po10", lag_s=2, lag_p=2, lag_o=1, groups=(4,) * 8, hold=2, spread=4,
                      spread_tail=2):
    bounds = [sum(groups[:g]) for g in range(len(groups) + 1)]
    first_held = len(groups) - 1 - hold
    shares = {}
    for g in range(len(groups)):
        if g == len(groups) - 1:
            slot, parts, step = 10 ** 6, spread_tail, 0
        elif g >= first_held:
            slot, parts, step = H_ + (g - first_held) * (lag_s + lag_p) // hold, spread_tail, 1
        else:
            slot, step = bounds[g + 1] - 1 + lag_s + lag_p + lag_o, 1
            parts = spread if slot < H_ else spread_tail
        for k in range(parts):
            cols = tuple(range(k * 8 // parts, (k + 1) * 8 // parts))
            shares.setdefault(slot + k * step, []).append(("o", bounds[g], bounds[g + 1], cols))
    sched = []
    for i in range(H_ + lag_s + lag_p):
        for ch in order:
            if ch in "012" and i < H_:
                sched.append(("proj", i, int(ch)))
            elif ch == "o":
                sched += shares.pop(i, [])
            elif ch == "s" and 0 <= i - lag_s < H_:
                sched.append(("s", i - lag_s))
            elif ch == "p" and 0 <= i - lag_s - lag_p < H_:
                sched.append(("pv", i - lag_s - lag_p))
    for slot in sorted(shares):
        sched += shares[slot]
    return sched


def _kernel(ax_hbm, wrt_hbm, wit_hbm, wrn_ref, win_ref, dmat_hbm, smat_hbm,
            bx_hbm, m0_ref, wq_hbm, wk_hbm, wv_hbm, wo_hbm, out_hbm,
            xg_ref, y_ref, t_ref, fw_ref, dmat_ref, smat_ref,
            w_ref, wo_ref, bxa_ref, bxp_ref, xp_ref, pre_ref, outb_ref,
            sem_ax, sem_fw, sem_c, sem_w, sem_wo, sem_bx, sem_outa, sem_outb):
    axu = ax_hbm.bitcast(u32)
    outu = out_hbm.bitcast(u32)
    w_hbm = [w.bitcast(u32) for w in (wq_hbm, wk_hbm, wv_hbm)]
    wou = wo_hbm.bitcast(u32)

    def ax_copies(c):
        pair = pl.ds(2 * c, 2)
        return [pltpu.make_async_copy(axu.at[:, c], xg_ref.at[c], sem_ax.at[c]),
                pltpu.make_async_copy(smat_hbm.at[pair], smat_ref.at[pair], sem_c.at[1 + c])]

    def w_copies(j, mi):
        return [pltpu.make_async_copy(w_hbm[mi].at[:, par * 16 + j], w_ref.at[mi, 2 * j + par],
                                      sem_w.at[3 * j + mi]) for par in range(2)]

    def outa_copy(c):
        return pltpu.make_async_copy(xg_ref.at[c], outu.at[:, c, pl.ds(0, D_)], sem_outa.at[0])

    dmat_copy = pltpu.make_async_copy(dmat_hbm, dmat_ref, sem_c.at[0])
    bxp_copy = pltpu.make_async_copy(bx_hbm.at[:, pl.ds(TOK_, PRE_)], bxp_ref, sem_bx.at[0])
    bxa_copy = pltpu.make_async_copy(bx_hbm.at[:, pl.ds(0, TOK_)], bxa_ref, sem_bx.at[1])
    fw_copies = []
    for ri, wh in enumerate((wrt_hbm, wit_hbm)):
        wu = wh.at[pl.ds(0, 512)].bitcast(u32)
        fw_copies.append([pltpu.make_async_copy(wu.at[:, pl.ds(k2 * 128, 128)], fw_ref.at[ri, k2], sem_fw.at[0])
                          for k2 in range(16)])
    wo_copies = [pltpu.make_async_copy(wou.at[:, pl.ds(n * 128, 128)], wo_ref.at[n], sem_wo.at[0])
                 for n in range(8)]

    def start_pair(j):
        for mi in range(3):
            for cp in w_copies(j, mi):
                cp.start()

    for c in range(8):
        for cp in ax_copies(c):
            cp.start()
        if c == 0:
            dmat_copy.start()

    def forward(i, carry):
        for u in range(2):
            for cp in ax_copies(2 * i + u):
                cp.wait()
        for j in range(AHEAD_):
            @pl.when(i == j + 1)
            def _():
                if j == 0:
                    bxp_copy.start()
                start_pair(j)
        for u in range(2):
            _feature_butterflies(xg_ref, y_ref, 2 * i + u, u)
            for par in range(2):
                _forward_matmuls(y_ref, t_ref, dmat_ref, smat_ref, 2 * (2 * i + u) + par, u, par)
        return carry

    dmat_copy.wait()
    lax.fori_loop(0, 4, forward, 0)

    def relayout(j, mi):
        for r in range(0, 512, 64):
            a = w_ref[mi, 2 * j, r:r + 64, :]
            b = w_ref[mi, 2 * j + 1, r:r + 64, :]
            w_ref[mi, 2 * j, r:r + 64, :] = (a & LO16) | (b << 16)
            w_ref[mi, 2 * j + 1, r:r + 64, :] = (a >> 16) | (b & HI16)

    bxp_copy.wait()
    for i in range(0, NSEG_, 2):
        v = jnp.concatenate([bxp_ref[i].astype(f32), bxp_ref[i + 1].astype(f32)], axis=0)
        xp_ref[i * 4:i * 4 + 8, :] = pltpu.bitcast(v.astype(bf16), u32)
    for cp in w_copies(0, 0):
        cp.wait()
    relayout(0, 0)

    def early_rows(j, carry, last=False):
        if not last:
            pl.when(j + AHEAD_ < H_ // 2)(lambda: start_pair(j + AHEAD_))
            for ri in range(2):
                @pl.when(j == ri)
                def _():
                    for cp in fw_copies[ri]:
                        cp.start()

            @pl.when(j == H_ // 2 - AHEAD_)
            def _():
                for cp in wo_copies:
                    cp.start()
                bxa_copy.start()
        for mi in (1, 2):
            for cp in w_copies(j, mi):
                cp.wait()
        if not last:
            for cp in w_copies(j + 1, 0):
                cp.wait()
        for mi in range(3):
            xp = _bf(xp_ref[...])
            for hh in range(2):
                pre_ref[mi, 2 * j + hh] = _dot(xp, _bf(w_ref[mi, 2 * j + hh]))
            if mi < 2:
                relayout(j, mi + 1)
            elif not last:
                relayout(j + 1, 0)
        return carry

    lax.fori_loop(0, H_ // 2 - 1, early_rows, 0)
    early_rows(H_ // 2 - 1, 0, last=True)

    for cps in fw_copies:
        for cp in cps:
            cp.wait()

    def filter_pair(m, carry):
        cls, g = m // 8, m % 8
        for odd in range(2):
            def get_w(k2):
                idx = pl.ds(g * 32 + cls, 8, stride=4)
                a, b = fw_ref[0, k2, idx, :], fw_ref[1, k2, idx, :]
                a, b = (a & HI16, b & HI16) if odd else (a << 16, b << 16)
                return pltpu.bitcast(a, f32), pltpu.bitcast(b, f32)

            _filter_rows(t_ref, pl.multiple_of((2 * cls + odd) * 64 + g * 8, 8), get_w)
        return carry

    lax.fori_loop(0, 32, filter_pair, 0)
    _filter_rows(t_ref, 512, lambda k2: tuple(
        jnp.broadcast_to(r[0:1, k2 * 128:(k2 + 1) * 128].astype(f32), (8, 128)) for r in (wrn_ref, win_ref)))

    def inverse(i, carry):
        for u in range(2):
            c = 2 * i + u
            res = [_inverse_matmuls(t_ref, dmat_ref, smat_ref, 2 * c + par) for par in range(2)]
            for a in range(8):
                words = pltpu.pack_elementwise([res[0][a], res[1][a]], packed_dtype=bf16)
                xg_ref[c, :, a * 128:(a + 1) * 128] = pltpu.bitcast(words, u32)
        for u in range(2):
            outa_copy(2 * i + u).start()
        return carry

    lax.fori_loop(0, 4, inverse, 0)

    for cp in wo_copies:
        cp.wait()
    bxa_copy.wait()
    sched = _segment_schedule()

    def segment(s, mem):
        early = pl.ds(pl.multiple_of(s * PRE_, PRE_), PRE_)
        row = lax.broadcasted_iota(jnp.int32, (L_, L_), 0)
        col = lax.broadcasted_iota(jnp.int32, (L_, L_), 1)
        mask = (row < M_) | (row >= col)
        xs = bxa_ref[s].astype(f32)
        hh = jnp.concatenate(
            [jnp.concatenate([mem[n], xs[:, n * 128:(n + 1) * 128]], axis=0) for n in range(8)], axis=1)
        proj, probs, att = {}, {}, {}
        acc = [None] * 8
        for op in sched:
            if op[0] == "proj":
                _, h, mi = op
                y = jnp.concatenate([_dot(hh, _bf(w_ref[mi, h])), pre_ref[mi, h, early, :]], axis=0)
                proj[h, mi] = y if mi == 0 else y.astype(bf16)
            elif op[0] == "s":
                h = op[1]
                qk = _dot_nt(proj.pop((h, 0)), proj.pop((h, 1)))
                sc = jnp.where(mask, qk * (DH_ ** -0.5 * LOG2E), -1e9 * LOG2E)
                e = jnp.exp2(sc - jnp.max(sc, axis=-1, keepdims=True))
                probs[h] = (e, pl.reciprocal(jnp.sum(e, axis=-1, keepdims=True)))
            elif op[0] == "pv":
                h = op[1]
                e, inv_sum = probs.pop(h)
                att[h] = _dot(e, proj.pop((h, 2))) * inv_sum
            else:
                _, h0, h1, cols = op
                og = jnp.concatenate([att[h] for h in range(h0, h1)], axis=1)
                for n in cols:
                    y = _dot(og, _bf(wo_ref[n, h0 * 64:h1 * 64, :]))
                    acc[n] = y if acc[n] is None else acc[n] + y
        for n in range(8):
            yb = acc[n][M_:L_].astype(bf16)
            outb_ref[2 * s, :, n * 128:(n + 1) * 128] = yb[0:16]
            outb_ref[2 * s + 1, :, n * 128:(n + 1) * 128] = yb[16:32]
        blk = pl.ds(2 * s, 2)
        pltpu.make_async_copy(outb_ref.at[blk], out_hbm.at[blk, :, pl.ds(D_, D_)], sem_outb.at[0]).start()
        return tuple(acc[n][0:M_] for n in range(8))

    m0 = m0_ref[...].astype(f32)
    lax.fori_loop(0, NSEG_, segment, tuple(m0[:, n * 128:(n + 1) * 128] for n in range(8)))
    for c in range(8):
        outa_copy(c).wait()
    pltpu.make_async_copy(outb_ref, out_hbm.at[:, :, pl.ds(D_, D_)], sem_outb.at[0]).wait()


@functools.partial(jax.jit, static_argnames=("B_seg_len",))
def pallas_concat_heads__spectral_gfnet__memory_aug_recurrent_mem_tr__prompt_kernel(
    A_x: jax.Array,
    A_w_r: jax.Array,
    A_w_i: jax.Array,
    B_x: jax.Array,
    B_mem0: jax.Array,
    B_Wq: jax.Array,
    B_Wk: jax.Array,
    B_Wv: jax.Array,
    B_Wo: jax.Array,
    B_seg_len: int,
):
    assert B_seg_len == SEG_
    assert A_x.shape == (1, S_, D_) and B_x.shape == (1, S_, D_)
    assert B_Wq.shape == (D_, H_, DH_) and B_mem0.shape == (1, M_, D_)
    wrt, wit = A_w_r.T, A_w_i.T
    hbm = pl.BlockSpec(memory_space=pltpu.HBM)
    nyquist = pl.BlockSpec((8, S_), lambda i: (64, 0))
    dma = pltpu.SemaphoreType.DMA
    out = pl.pallas_call(
        _kernel,
        grid=(1,),
        out_shape=jax.ShapeDtypeStruct((128, 16, 2 * D_), bf16),
        in_specs=[hbm, hbm, hbm, nyquist, nyquist, hbm, hbm,
                  hbm, pl.BlockSpec((M_, D_), lambda i: (0, 0)), hbm, hbm, hbm, hbm],
        out_specs=hbm,
        scratch_shapes=[
            pltpu.VMEM((8, 128, D_), u32),
            pltpu.VMEM((2, 2, 11, 64, 128), u32),
            pltpu.VMEM((2, 16, KR_, 128), f32),
            pltpu.VMEM((2, 16, 256, 128), u32),
            pltpu.VMEM(_DMAT.shape, u32),
            pltpu.VMEM(_SMAT.shape, u32),
            pltpu.VMEM((3, H_, D_ // 2, DH_), u32),
            pltpu.VMEM((8, H_ * DH_ // 2, 128), u32),
            pltpu.VMEM((NSEG_, TOK_, D_), bf16),
            pltpu.VMEM((NSEG_, PRE_, D_), bf16),
            pltpu.VMEM((NSEG_ * PRE_ // 2, D_), u32),
            pltpu.VMEM((3, H_, NSEG_ * PRE_, DH_), f32),
            pltpu.VMEM((128, 16, D_), bf16),
            dma((8,)), dma((1,)), dma((9,)), dma((3 * H_ // 2,)), dma((1,)), dma((2,)), dma((1,)), dma((1,)),
        ],
        compiler_params=pltpu.CompilerParams(
            dimension_semantics=("arbitrary",),
            vmem_limit_bytes=120 * 1024 * 1024,
            flags={"XLA_TPU_EVENLY_DISTRIBUTE_CRITICAL_NODES": True}),
    )(A_x.reshape(128, 16, D_), wrt, wit, wrt, wit, _DMAT, _SMAT,
      B_x.reshape(NSEG_, SEG_, D_), B_mem0.reshape(M_, D_),
      B_Wq.reshape(D_ // 2, 2 * H_, DH_), B_Wk.reshape(D_ // 2, 2 * H_, DH_), B_Wv.reshape(D_ // 2, 2 * H_, DH_),
      B_Wo.reshape(H_ * DH_, D_))
    return out.reshape(1, S_, 2 * D_)
```

```python
import functools

import jax
import jax.numpy as jnp
import ml_dtypes
import numpy as np
from jax import lax
import jax.experimental.pallas as pl
import jax.experimental.pallas.tpu as pltpu

S_, D_, H_, DH_, M_, SEG_ = 2048, 1024, 32, 128, 8, 32
L_ = M_ + SEG_
NSEG_ = S_ // SEG_
PRE_ = 8
TOK_ = SEG_ - PRE_
KR_ = 520
AHEAD_ = 4
NFULL_ = 4
NPAIR_ = (H_ - NFULL_) // 2
UNROLL_ = 4
f32, bf16, u32 = jnp.float32, jnp.bfloat16, jnp.uint32
HI16 = np.uint32(0xFFFF0000)
LO16 = np.uint32(0xFFFF)
R2 = float(np.sqrt(0.5))
LOG2E = float(np.log2(np.e))


def _dft_constants():
    th = 2 * np.pi / D_
    b = np.arange(128)
    j = np.arange(64)

    def cs(k):
        ang = th * ((k[:, None] * b[None, :]) % D_)
        return np.cos(ang), np.sin(ang)

    c0, s0 = cs(8 * j)
    c4, s4 = cs(4 + 8 * j)
    alt = (-1.0) ** b
    nyq = np.zeros((16, 128))
    nyq[0] = alt
    l0 = np.concatenate([c0, -s0], 0)
    l4 = np.concatenate([c4, -s4], 0)
    i0 = l0.copy()
    i0[0] *= 0.5
    i0[64] = 0.5 * alt
    fwd, inv = [l4], [i0]
    lower = np.where(np.arange(128) < 64, 1.0, -1.0)[:, None]
    for r in (1, 2, 3):
        ca, sa = cs(r + 8 * j)
        cb, sb = cs(8 - r + 8 * j)
        c = np.concatenate([ca, cb], 0)
        d = np.concatenate([-sa, sb], 0)
        fwd += [c, c + d, (d - c) * lower]
        inv += [d - c]
    n1 = np.arange(128)
    seq = []
    for n2 in range(16):
        ang = 2 * np.pi / S_ * (((16 * n1 + n2)[:, None] * n1[None, :]) % S_)
        c, d = np.cos(ang) * 2.0 ** -10, -np.sin(ang) * 2.0 ** -10
        seq.append(np.stack([c, d - c, c + d]))
        inv.append(d)

    def words(m):
        u = m.astype(ml_dtypes.bfloat16).view(np.uint16).astype(np.uint32)
        return u[..., 0::2, :] | (u[..., 1::2, :] << 16)

    return words(np.concatenate(fwd + [l0, nyq], 0)), words(np.stack(seq)), words(np.stack(inv))


_DMAT, _SMAT, _IMAT = _dft_constants()


def _bf(words):
    return pltpu.bitcast(words, bf16)


def _dot_nt(a, b):
    return lax.dot_general(a, b, (((1,), (1,)), ((), ())), preferred_element_type=f32)


def _dot(a, b):
    return jnp.dot(a, b, preferred_element_type=f32)


def _radix4(xs, sgn):
    (ar, ai), (br, bi), (cr, ci), (dr, di) = xs
    t0r, t0i = ar + cr, ai + ci
    t1r, t1i = ar - cr, ai - ci
    t2r, t2i = br + dr, bi + di
    t3r, t3i = br - dr, bi - di
    y0 = (t0r + t2r, t0i + t2i)
    y2 = (t0r - t2r, t0i - t2i)
    ym = (t1r + t3i, t1i - t3r)
    yp = (t1r - t3i, t1i + t3r)
    return [y0, ym, y2, yp] if sgn < 0 else [y0, yp, y2, ym]


def _twiddle16(z, e, sgn):
    r, i = z
    if e == 0:
        return z
    if e == 4:
        return (-i, r) if sgn > 0 else (i, -r)
    if e == 2:
        return ((r - i) * R2, (r + i) * R2) if sgn > 0 else ((r + i) * R2, (i - r) * R2)
    if e == 6:
        return ((-r - i) * R2, (r - i) * R2) if sgn > 0 else ((i - r) * R2, (-r - i) * R2)
    c = float(np.cos(2 * np.pi * e / 16))
    s = float(sgn * np.sin(2 * np.pi * e / 16))
    return (r * c - i * s, r * s + i * c)


def _fft16(xs, sgn):
    a = [_radix4([xs[4 * p + q] for p in range(4)], sgn) for q in range(4)]
    out = [None] * 16
    for u in range(4):
        y = _radix4([_twiddle16(a[q][u], q * u, sgn) for q in range(4)], sgn)
        for v in range(4):
            out[u + 4 * v] = y[v]
    return out


def _forward_rows(xg_ref, t_ref, dmat_ref, smat_ref, c, par):
    n2 = 2 * c + par

    def dm(i):
        return _bf(dmat_ref[i * 64:(i + 1) * 64, :])

    def butterflies(odd):
        outs = []
        for r0 in range(0, 128, 16):
            w = [xg_ref[c, r0:r0 + 16, a * 128:(a + 1) * 128] for a in range(8)]
            xa = [pltpu.bitcast((v << 16) if par == 0 else (v & HI16), f32) for v in w]
            if odd:
                t1, t3, t5, t7 = xa[0] - xa[4], xa[2] - xa[6], xa[1] - xa[5], xa[3] - xa[7]
                u, v = (t5 - t7) * R2, (t5 + t7) * -R2
                p1, q1, p3, q3 = t1 + u, v - t3, t1 - u, t3 + v
                ys = [p1, q1, p1 + q1, p3, q3, p3 + q3]
            else:
                t0, t2, t4, t6 = xa[0] + xa[4], xa[2] + xa[6], xa[1] + xa[5], xa[3] + xa[7]
                e, o = t0 + t2, t4 + t6
                p2, q2 = t0 - t2, t6 - t4
                ys = [e + o, e - o, p2, q2, p2 + q2]
            outs.append([yv.astype(bf16) for yv in ys])
        return [jnp.concatenate(col, axis=0) for col in zip(*outs)]

    def feature_stage(r, ys):
        if r == 0:
            z0 = _dot_nt(_bf(dmat_ref[10 * 64:10 * 64 + 72, :]), ys[0])
            z4 = _dot_nt(dm(0), ys[1])
            return (jnp.concatenate([z0[0:64], z4[0:64]], axis=0),
                    jnp.concatenate([z0[64:128], z4[64:128]], axis=0), z0[128:136])
        p, q, pq = ys
        k1 = _dot_nt(dm(3 * r - 2), pq)
        k2 = _dot_nt(dm(3 * r), p)
        k3 = _dot_nt(dm(3 * r - 1), q)
        return k1 - k3, jnp.concatenate([k1[0:64] + k2[0:64], k2[64:128] - k1[64:128]], axis=0), None

    def sequence_stage(r, zr, zi, zn):
        zs = zr + zi
        if zn is not None:
            zs, zr = jnp.concatenate([zs, zn], axis=0), jnp.concatenate([zr, zn], axis=0)
        k1 = _dot(zs, _bf(smat_ref[n2, 0]))
        k2 = _dot(zr, _bf(smat_ref[n2, 1]))
        k3 = _dot(zi, _bf(smat_ref[n2, 2]))
        re, im = k1[0:128] - k3, k1 + k2
        ra, rb = (0, 4) if r == 0 else (r, 8 - r)
        for ri, v in enumerate((re, im)):
            t_ref[ri, n2, 64 * ra:64 * ra + 64, :] = v[0:64]
            t_ref[ri, n2, 64 * rb:64 * rb + 64, :] = v[64:128]
        if zn is not None:
            t_ref[0, n2, 512:KR_, :] = k1[128:136]
            t_ref[1, n2, 512:KR_, :] = im[128:136]

    ye = butterflies(False)
    z0 = feature_stage(0, ye[0:2])
    z2 = feature_stage(2, ye[2:5])
    yo = butterflies(True)
    sequence_stage(0, *z0)
    z1 = feature_stage(1, yo[0:3])
    sequence_stage(2, *z2)
    z3 = feature_stage(3, yo[3:6])
    sequence_stage(1, *z1)
    sequence_stage(3, *z3)


def _inverse_rows(t_ref, dmat_ref, smat_ref, imat_ref, n2):
    def dm(i):
        return _bf(dmat_ref[i * 64:(i + 1) * 64, :])

    row = lax.broadcasted_iota(jnp.int32, (8, 128), 0)
    lane = lax.broadcasted_iota(jnp.int32, (1, 128), 1)
    sgn = jnp.where(lane < 64, 1.0, -1.0).astype(f32)
    mcd = jnp.concatenate([_bf(smat_ref[n2, 0]), _bf(imat_ref[4 + n2])], axis=1)
    vr, vi = t_ref[0, n2, 0:64, :], t_ref[1, n2, 0:64, :]
    nr, ni = t_ref[0, n2, 512:KR_, :], t_ref[1, n2, 512:KR_, :]
    vi0 = jnp.concatenate([jnp.where(row == 0, nr, vi[0:8]), vi[8:64]], axis=0)
    vr0 = jnp.concatenate([jnp.where(row == 0, ni, -vr[0:8]), -vr[8:64]], axis=0)
    ra = jnp.concatenate([jnp.concatenate([vr, vi0], axis=0),
                          jnp.concatenate([vi, vr0], axis=0)], axis=1).astype(bf16)
    ta = _dot_nt(mcd, ra)
    vr, vi = t_ref[0, n2, 256:320, :], t_ref[1, n2, 256:320, :]
    rb = jnp.concatenate([jnp.concatenate([vr, vi], axis=0),
                          jnp.concatenate([vi, -vr], axis=0)], axis=1).astype(bf16)
    tb = _dot_nt(mcd, rb)
    us = []
    for r in (1, 2, 3):
        vr, vi = [jnp.concatenate([t_ref[ri, n2, 64 * r:64 * r + 64, :],
                                   t_ref[ri, n2, 64 * (8 - r):64 * (9 - r), :]], axis=0) for ri in range(2)]
        k1 = _dot_nt(_bf(smat_ref[n2, 0]), (vr + vi).astype(bf16))
        k2 = _dot_nt(_bf(smat_ref[n2, 2]), vr.astype(bf16))
        k3 = _dot_nt(_bf(smat_ref[n2, 1]), vi.astype(bf16))
        us.append((k1 + k3, (k1 - k2) * sgn))
    g0 = _dot(ta, _bf(imat_ref[0]))
    g4 = _dot(tb, dm(0))
    hr, hi = [], []
    for r in (1, 2, 3):
        ur, ui = us[r - 1]
        k1 = _dot(ur + ui, dm(3 * r - 2))
        k2 = _dot(ur, dm(3 * r - 1))
        k3 = _dot(ui, _bf(imat_ref[r]))
        hr.append(k1 + k3)
        hi.append(k1 - k2)
    ep, em = g0 + g4, g0 - g4
    s13 = hr[0] + hr[2]
    d13 = hi[0] - hi[2]
    p = ((hr[0] - hi[0]) - (hr[2] + hi[2])) * R2
    q = ((hr[2] - hi[2]) - (hr[0] + hi[0])) * R2
    e1, e2 = ep + hr[1], ep - hr[1]
    e3, e4 = em - hi[1], em + hi[1]
    return [e1 + s13, e3 + p, e2 - d13, e4 + q, e1 - s13, e3 - p, e2 + d13, e4 - q]


def _filter_rows(t_ref, row0, get_w):
    rows = pl.ds(row0, 8)
    xf = _fft16([(t_ref[0, n2, rows, :], t_ref[1, n2, rows, :]) for n2 in range(16)], -1)
    prod = []
    for k2 in range(16):
        wr, wi = get_w(k2)
        xr, xi = xf[k2]
        prod.append((xr * wr - xi * wi, xr * wi + xi * wr))
    vs = _fft16(prod, +1)
    for n2 in range(16):
        t_ref[0, n2, rows, :] = vs[n2][0]
        t_ref[1, n2, rows, :] = vs[n2][1]


def _segment_schedule(order="ps2o10", lag_s=2, lag_p=2, lag_o=0, groups=(4, 4, 4, 4, 4, 4, 2, 2, 2, 2),
                      hold=5, spread=8, spread_tail=2):
    bounds = [sum(groups[:g]) for g in range(len(groups) + 1)]
    first_held = len(groups) - 1 - hold
    shares = {}
    for g in range(len(groups)):
        if g == len(groups) - 1:
            slot, parts, step = 10 ** 6, spread_tail, 0
        elif g >= first_held:
            slot, parts, step = H_ + (g - first_held) * (lag_s + lag_p) // hold, spread_tail, 1
        else:
            slot, step = bounds[g + 1] - 1 + lag_s + lag_p + lag_o, 1
            parts = spread if slot < H_ else spread_tail
        for k in range(parts):
            cols = tuple(range(k * 8 // parts, (k + 1) * 8 // parts))
            shares.setdefault(slot + k * step, []).append(("o", bounds[g], bounds[g + 1], cols))
    sched = []
    for i in range(H_ + lag_s + lag_p):
        for ch in order:
            if ch in "012" and i < H_:
                sched.append(("proj", i, int(ch)))
            elif ch == "o":
                sched += shares.pop(i, [])
            elif ch == "s" and 0 <= i - lag_s < H_:
                sched.append(("s", i - lag_s))
            elif ch == "p" and 0 <= i - lag_s - lag_p < H_:
                sched.append(("pv", i - lag_s - lag_p))
    for slot in sorted(shares):
        sched += shares[slot]
    return sched


def _kernel(ax_hbm, wrt_hbm, wit_hbm, dmat_hbm, smat_hbm, imat_hbm,
            bx_hbm, m0_hbm, wq_hbm, wk_hbm, wv_hbm, wo_hbm, out_hbm,
            xg_ref, t_ref, fw_ref, fn_ref, dmat_ref, smat_ref, imat_ref,
            w_ref, wo_ref, bxa_ref, bxp_ref, m0_ref, xp_ref, pre_ref, outb_ref,
            sem_ax, sem_c, sem_fw, sem_w, sem_late, sem_bx, sem_outa, sem_outb):
    axu = ax_hbm.bitcast(u32)
    outu = out_hbm.bitcast(u32)
    w_hbm = [w.bitcast(u32) for w in (wq_hbm, wk_hbm, wv_hbm)]
    wou = wo_hbm.bitcast(u32)

    def ax_copies(c):
        pair = pl.ds(2 * c, 2)
        return [pltpu.make_async_copy(axu.at[:, c], xg_ref.at[c], sem_ax.at[c]),
                pltpu.make_async_copy(smat_hbm.at[pair], smat_ref.at[pair], sem_c.at[1 + c])]

    def w_copies(j, mi):
        return [pltpu.make_async_copy(w_hbm[mi].at[:, par * 16 + j], w_ref.at[mi, 2 * j + par],
                                      sem_w.at[3 * j + mi]) for par in range(2)]

    def outa_copy(c):
        return pltpu.make_async_copy(xg_ref.at[c], outu.at[:, c, pl.ds(0, D_)], sem_outa.at[0])

    def outb_copy(s0, n):
        blk = pl.ds(2 * s0, 2 * n)
        return pltpu.make_async_copy(outb_ref.at[blk], out_hbm.at[blk, :, pl.ds(D_, D_)], sem_outb.at[0])

    dmat_copy = pltpu.make_async_copy(dmat_hbm, dmat_ref, sem_c.at[0])
    bxp_copy = pltpu.make_async_copy(bx_hbm.at[:, pl.ds(TOK_, PRE_)], bxp_ref, sem_bx.at[0])
    fwu = [wh.at[pl.ds(0, 512)].bitcast(u32) for wh in (wrt_hbm, wit_hbm)]

    def fw_copy(ri, k2):
        lanes = pl.ds(pl.multiple_of(k2 * 128, 128), 128)
        return pltpu.make_async_copy(fwu[ri].at[:, lanes], fw_ref.at[ri, k2, pl.ds(0, 256)], sem_fw.at[0])

    inv_copies = [pltpu.make_async_copy(wh.at[pl.ds(512, 1)], fn_ref.at[ri], sem_fw.at[1])
                  for ri, wh in enumerate((wrt_hbm, wit_hbm))]
    inv_copies.append(pltpu.make_async_copy(imat_hbm, imat_ref, sem_fw.at[1]))

    def wo_copy(n):
        lanes = pl.ds(pl.multiple_of(n * 128, 128), 128)
        return pltpu.make_async_copy(wou.at[:, lanes], wo_ref.at[n], sem_late.at[0])

    late_copies = [pltpu.make_async_copy(bx_hbm.at[:, pl.ds(0, TOK_)], bxa_ref, sem_late.at[1]),
                   pltpu.make_async_copy(m0_hbm, m0_ref, sem_late.at[1])]

    def start_pair(j):
        for mi in range(3):
            for cp in w_copies(j, mi):
                cp.start()

    for c in range(8):
        for cp in ax_copies(c):
            cp.start()
        if c == 0:
            dmat_copy.start()

    def forward(i, carry):
        for u in range(2):
            for cp in ax_copies(2 * i + u):
                cp.wait()
        for u in range(2):
            for par in range(2):
                _forward_rows(xg_ref, t_ref, dmat_ref, smat_ref, 2 * i + u, par)
        pl.when(i == 0)(bxp_copy.start)
        start_pair(i)
        return carry

    dmat_copy.wait()
    lax.fori_loop(0, 4, forward, 0)

    def relayout(j, mi):
        for r in range(0, 512, 64):
            a = w_ref[mi, 2 * j, r:r + 64, :]
            b = w_ref[mi, 2 * j + 1, r:r + 64, :]
            w_ref[mi, 2 * j, r:r + 64, :] = (a & LO16) | (b << 16)
            w_ref[mi, 2 * j + 1, r:r + 64, :] = (a >> 16) | (b & HI16)

    bxp_copy.wait()
    for i in range(0, NSEG_, 2):
        v = jnp.concatenate([bxp_ref[i].astype(f32), bxp_ref[i + 1].astype(f32)], axis=0)
        xp_ref[i * 4:i * 4 + 8, :] = pltpu.bitcast(v.astype(bf16), u32)
    for cp in w_copies(0, 0):
        cp.wait()
    relayout(0, 0)

    def early_rows(j, carry, last=False):
        todo = [(j, 1), (j, 2)]
        if last:
            todo += [(jj, mi) for jj in range(NPAIR_, H_ // 2) for mi in range(3)]
            for cp in late_copies:
                cp.start()
        else:
            todo += [(j + 1, 0)]
        for it in todo:
            for cp in w_copies(*it):
                cp.wait()
        for mi in range(3):
            xp = _bf(xp_ref[...])
            for hh in range(2):
                pre_ref[mi, 2 * j + hh] = _dot(xp, _bf(w_ref[mi, 2 * j + hh]))
            for it in todo[mi::3]:
                relayout(*it)
        if not last:
            pl.when(j + AHEAD_ < H_ // 2)(lambda: start_pair(j + AHEAD_))

            @pl.when(j < 8)
            def _():
                for ri in range(2):
                    for k in range(2):
                        fw_copy(ri, 2 * j + k).start()

            pl.when(j >= NPAIR_ - 9)(lambda: wo_copy(j - (NPAIR_ - 9)).start())
        return carry

    for cp in inv_copies:
        cp.start()
    lax.fori_loop(0, NPAIR_ - 1, early_rows, 0)
    early_rows(NPAIR_ - 1, 0, last=True)

    fw_all = fw_ref.at[:, :, pl.ds(0, 256)]
    pltpu.make_async_copy(fw_all, fw_all, sem_fw.at[0]).wait()
    for cp in inv_copies:
        cp.wait()

    def filter_pair(m, carry):
        cls, g = m // 8, m % 8
        for odd in range(2):
            def get_w(k2):
                idx = pl.ds(g * 32 + cls, 8, stride=4)
                a, b = fw_ref[0, k2, idx, :], fw_ref[1, k2, idx, :]
                a, b = (a & HI16, b & HI16) if odd else (a << 16, b << 16)
                return pltpu.bitcast(a, f32), pltpu.bitcast(b, f32)

            _filter_rows(t_ref, pl.multiple_of((2 * cls + odd) * 64 + g * 8, 8), get_w)
        return carry

    lax.fori_loop(0, 32, filter_pair, 0)
    _filter_rows(t_ref, 512, lambda k2: tuple(
        jnp.broadcast_to(fn_ref[ri, :, k2 * 128:(k2 + 1) * 128].astype(f32), (8, 128)) for ri in range(2)))

    def inverse(i, carry):
        for u in range(2):
            c = 2 * i + u
            res = [_inverse_rows(t_ref, dmat_ref, smat_ref, imat_ref, 2 * c + par) for par in range(2)]
            for a in range(8):
                words = pltpu.pack_elementwise([res[0][a], res[1][a]], packed_dtype=bf16)
                xg_ref[c, :, a * 128:(a + 1) * 128] = pltpu.bitcast(words, u32)
        for u in range(2):
            outa_copy(2 * i + u).start()
        return carry

    lax.fori_loop(0, 4, inverse, 0)

    pltpu.make_async_copy(wo_ref, wo_ref, sem_late.at[0]).wait()
    for cp in late_copies:
        cp.wait()
    sched = _segment_schedule()

    def head(t):
        return (t - NFULL_) % H_

    def segment(s, mem):
        early = pl.ds(pl.multiple_of(s * PRE_, PRE_), PRE_)
        row = lax.broadcasted_iota(jnp.int32, (L_, L_), 0)
        col = lax.broadcasted_iota(jnp.int32, (L_, L_), 1)
        mask = (row < M_) | (row >= col)
        xs = bxa_ref[s].astype(f32)
        h32 = jnp.concatenate(
            [jnp.concatenate([mem[n], xs[:, n * 128:(n + 1) * 128]], axis=0) for n in range(8)], axis=1)
        h40 = jnp.concatenate([h32, bxp_ref[s].astype(f32)], axis=0)
        proj, probs, att = {}, {}, {}
        acc = [None] * 8
        for op in sched:
            if op[0] == "proj":
                _, t, mi = op
                w = _bf(w_ref[mi, head(t)])
                if t < NFULL_:
                    y = _dot(h40, w)
                else:
                    y = jnp.concatenate([_dot(h32, w), pre_ref[mi, head(t), early, :]], axis=0)
                proj[t, mi] = y if mi == 0 else y.astype(bf16)
            elif op[0] == "s":
                t = op[1]
                qk = _dot_nt(proj.pop((t, 0)), proj.pop((t, 1)))
                sc = jnp.where(mask, qk * (DH_ ** -0.5 * LOG2E), -1e9 * LOG2E)
                e = jnp.exp2(sc - jnp.max(sc, axis=-1, keepdims=True))
                probs[t] = (e, pl.reciprocal(jnp.sum(e, axis=-1, keepdims=True)))
            elif op[0] == "pv":
                t = op[1]
                e, inv_sum = probs.pop(t)
                att[t] = _dot(e, proj.pop((t, 2))) * inv_sum
            else:
                _, t0, t1, cols = op
                og = jnp.concatenate([att[t] for t in range(t0, t1)], axis=1)
                for n in cols:
                    y = _dot(og, _bf(wo_ref[n, head(t0) * 64:(head(t1 - 1) + 1) * 64, :]))
                    acc[n] = y if acc[n] is None else acc[n] + y
        for n in range(8):
            yb = acc[n][M_:].astype(bf16)
            outb_ref[2 * s, :, n * 128:(n + 1) * 128] = yb[0:16]
            outb_ref[2 * s + 1, :, n * 128:(n + 1) * 128] = yb[16:32]
        return tuple(acc[n][0:M_] for n in range(8))

    def segments(i, mem):
        for u in range(UNROLL_):
            mem = segment(i * UNROLL_ + u, mem)
        outb_copy(i * UNROLL_, UNROLL_).start()
        return mem

    m0 = m0_ref[...].astype(f32)
    lax.fori_loop(0, NSEG_ // UNROLL_, segments, tuple(m0[:, n * 128:(n + 1) * 128] for n in range(8)))
    for c in range(8):
        outa_copy(c).wait()
    outb_copy(0, NSEG_).wait()


@functools.partial(jax.jit, static_argnames=("B_seg_len",))
def pallas_concat_heads__spectral_gfnet__memory_aug_recurrent_mem_tr__prompt_kernel(
    A_x: jax.Array,
    A_w_r: jax.Array,
    A_w_i: jax.Array,
    B_x: jax.Array,
    B_mem0: jax.Array,
    B_Wq: jax.Array,
    B_Wk: jax.Array,
    B_Wv: jax.Array,
    B_Wo: jax.Array,
    B_seg_len: int,
):
    assert B_seg_len == SEG_
    assert A_x.shape == (1, S_, D_) and B_x.shape == (1, S_, D_)
    assert B_Wq.shape == (D_, H_, DH_) and B_mem0.shape == (1, M_, D_)
    hbm = pl.BlockSpec(memory_space=pltpu.HBM)
    dma = pltpu.SemaphoreType.DMA
    out = pl.pallas_call(
        _kernel,
        out_shape=jax.ShapeDtypeStruct((128, 16, 2 * D_), bf16),
        in_specs=[hbm] * 12,
        out_specs=hbm,
        scratch_shapes=[
            pltpu.VMEM((8, 128, D_), u32),
            pltpu.VMEM((2, 16, KR_, 128), f32),
            pltpu.VMEM((2, 16, 264, 128), u32),
            pltpu.VMEM((2, 1, S_), bf16),
            pltpu.VMEM(_DMAT.shape, u32),
            pltpu.VMEM(_SMAT.shape, u32),
            pltpu.VMEM(_IMAT.shape, u32),
            pltpu.VMEM((3, H_, D_ // 2, DH_), u32),
            pltpu.VMEM((8, H_ * DH_ // 2, 128), u32),
            pltpu.VMEM((NSEG_, TOK_, D_), bf16),
            pltpu.VMEM((NSEG_, PRE_, D_), bf16),
            pltpu.VMEM((M_, D_), bf16),
            pltpu.VMEM((NSEG_ * PRE_ // 2, D_), u32),
            pltpu.VMEM((3, H_ - NFULL_, NSEG_ * PRE_, DH_), f32),
            pltpu.VMEM((128, 16, D_), bf16),
            dma((8,)), dma((9,)), dma((2,)), dma((3 * H_ // 2,)), dma((2,)), dma((1,)), dma((1,)), dma((1,)),
        ],
        compiler_params=pltpu.CompilerParams(
            vmem_limit_bytes=120 * 1024 * 1024,
            flags={"XLA_TPU_EVENLY_DISTRIBUTE_CRITICAL_NODES": True}),
    )(A_x.reshape(128, 16, D_), A_w_r.T, A_w_i.T, _DMAT, _SMAT, _IMAT,
      B_x.reshape(NSEG_, SEG_, D_), B_mem0.reshape(M_, D_),
      B_Wq.reshape(D_ // 2, 2 * H_, DH_), B_Wk.reshape(D_ // 2, 2 * H_, DH_), B_Wv.reshape(D_ // 2, 2 * H_, DH_),
      B_Wo.reshape(H_ * DH_, D_))
    return out.reshape(1, S_, 2 * D_)
```

```python
import functools

import jax
import jax.numpy as jnp
import ml_dtypes
import numpy as np
from jax import lax
import jax.experimental.pallas as pl
import jax.experimental.pallas.tpu as pltpu

S_, D_, H_, DH_, M_, SEG_ = 2048, 1024, 32, 128, 8, 32
L_ = M_ + SEG_
NSEG_ = S_ // SEG_
PRE_ = 8
TOK_ = SEG_ - PRE_
KR_ = 520
AHEAD_ = 4
NFULL_ = 4
NPAIR_ = (H_ - NFULL_) // 2
UNROLL_ = 4
f32, bf16, u32 = jnp.float32, jnp.bfloat16, jnp.uint32
HI16 = np.uint32(0xFFFF0000)
LO16 = np.uint32(0xFFFF)
R2 = float(np.sqrt(0.5))
LOG2E = float(np.log2(np.e))


def _dft_constants():
    th = 2 * np.pi / D_
    b = np.arange(128)
    j = np.arange(64)

    def cs(k):
        ang = th * ((k[:, None] * b[None, :]) % D_)
        return np.cos(ang), np.sin(ang)

    c0, s0 = cs(8 * j)
    c4, s4 = cs(4 + 8 * j)
    alt = (-1.0) ** b
    nyq = np.zeros((16, 128))
    nyq[0] = alt
    l0 = np.concatenate([c0, -s0], 0)
    l4 = np.concatenate([c4, -s4], 0)
    i0 = l0.copy()
    i0[0] *= 0.5
    i0[64] = 0.5 * alt
    fwd, inv = [l4], [i0]
    lower = np.where(np.arange(128) < 64, 1.0, -1.0)[:, None]
    for r in (1, 2, 3):
        ca, sa = cs(r + 8 * j)
        cb, sb = cs(8 - r + 8 * j)
        c = np.concatenate([ca, cb], 0)
        d = np.concatenate([-sa, sb], 0)
        fwd += [c, c + d, (d - c) * lower]
        inv += [d - c]
    n1 = np.arange(128)
    seq = []
    for n2 in range(16):
        ang = 2 * np.pi / S_ * (((16 * n1 + n2)[:, None] * n1[None, :]) % S_)
        c, d = np.cos(ang) * 2.0 ** -10, -np.sin(ang) * 2.0 ** -10
        seq.append(np.stack([c, d - c, c + d]))
        inv.append(d)

    def words(m):
        u = m.astype(ml_dtypes.bfloat16).view(np.uint16).astype(np.uint32)
        return u[..., 0::2, :] | (u[..., 1::2, :] << 16)

    return words(np.concatenate(fwd + [l0, nyq], 0)), words(np.stack(seq)), words(np.stack(inv))


_DMAT, _SMAT, _IMAT = _dft_constants()


def _bf(words):
    return pltpu.bitcast(words, bf16)


def _dot_nt(a, b):
    return lax.dot_general(a, b, (((1,), (1,)), ((), ())), preferred_element_type=f32)


def _dot(a, b):
    return jnp.dot(a, b, preferred_element_type=f32)


def _radix4(xs, sgn):
    (ar, ai), (br, bi), (cr, ci), (dr, di) = xs
    t0r, t0i = ar + cr, ai + ci
    t1r, t1i = ar - cr, ai - ci
    t2r, t2i = br + dr, bi + di
    t3r, t3i = br - dr, bi - di
    y0 = (t0r + t2r, t0i + t2i)
    y2 = (t0r - t2r, t0i - t2i)
    ym = (t1r + t3i, t1i - t3r)
    yp = (t1r - t3i, t1i + t3r)
    return [y0, ym, y2, yp] if sgn < 0 else [y0, yp, y2, ym]


def _twiddle16(z, e, sgn):
    r, i = z
    if e == 0:
        return z
    if e == 4:
        return (-i, r) if sgn > 0 else (i, -r)
    if e == 2:
        return ((r - i) * R2, (r + i) * R2) if sgn > 0 else ((r + i) * R2, (i - r) * R2)
    if e == 6:
        return ((-r - i) * R2, (r - i) * R2) if sgn > 0 else ((i - r) * R2, (-r - i) * R2)
    c = float(np.cos(2 * np.pi * e / 16))
    s = float(sgn * np.sin(2 * np.pi * e / 16))
    return (r * c - i * s, r * s + i * c)


def _fft16(xs, sgn):
    a = [_radix4([xs[4 * p + q] for p in range(4)], sgn) for q in range(4)]
    out = [None] * 16
    for u in range(4):
        y = _radix4([_twiddle16(a[q][u], q * u, sgn) for q in range(4)], sgn)
        for v in range(4):
            out[u + 4 * v] = y[v]
    return out


def _forward_rows(xg_ref, t_ref, dmat_ref, smat_ref, c, par):
    n2 = 2 * c + par

    def dm(i):
        return _bf(dmat_ref[i * 64:(i + 1) * 64, :])

    def butterflies(odd):
        outs = []
        for r0 in range(0, 128, 16):
            w = [xg_ref[c, r0:r0 + 16, a * 128:(a + 1) * 128] for a in range(8)]
            xa = [pltpu.bitcast((v << 16) if par == 0 else (v & HI16), f32) for v in w]
            if odd:
                t1, t3, t5, t7 = xa[0] - xa[4], xa[2] - xa[6], xa[1] - xa[5], xa[3] - xa[7]
                u, v = (t5 - t7) * R2, (t5 + t7) * -R2
                p1, q1, p3, q3 = t1 + u, v - t3, t1 - u, t3 + v
                ys = [p1, q1, p1 + q1, p3, q3, p3 + q3]
            else:
                t0, t2, t4, t6 = xa[0] + xa[4], xa[2] + xa[6], xa[1] + xa[5], xa[3] + xa[7]
                e, o = t0 + t2, t4 + t6
                p2, q2 = t0 - t2, t6 - t4
                ys = [e + o, e - o, p2, q2, p2 + q2]
            outs.append([yv.astype(bf16) for yv in ys])
        return [jnp.concatenate(col, axis=0) for col in zip(*outs)]

    def feature_stage(r, ys):
        if r == 0:
            z0 = _dot_nt(_bf(dmat_ref[10 * 64:10 * 64 + 72, :]), ys[0])
            z4 = _dot_nt(dm(0), ys[1])
            return (jnp.concatenate([z0[0:64], z4[0:64]], axis=0),
                    jnp.concatenate([z0[64:128], z4[64:128]], axis=0), z0[128:136])
        p, q, pq = ys
        k1 = _dot_nt(dm(3 * r - 2), pq)
        k2 = _dot_nt(dm(3 * r), p)
        k3 = _dot_nt(dm(3 * r - 1), q)
        return k1 - k3, jnp.concatenate([k1[0:64] + k2[0:64], k2[64:128] - k1[64:128]], axis=0), None

    def sequence_stage(r, zr, zi, zn):
        zs = zr + zi
        if zn is not None:
            zs, zr = jnp.concatenate([zs, zn], axis=0), jnp.concatenate([zr, zn], axis=0)
        k1 = _dot(zs, _bf(smat_ref[n2, 0]))
        k2 = _dot(zr, _bf(smat_ref[n2, 1]))
        k3 = _dot(zi, _bf(smat_ref[n2, 2]))
        re, im = k1[0:128] - k3, k1 + k2
        ra, rb = (0, 4) if r == 0 else (r, 8 - r)
        for ri, v in enumerate((re, im)):
            t_ref[ri, n2, 64 * ra:64 * ra + 64, :] = v[0:64]
            t_ref[ri, n2, 64 * rb:64 * rb + 64, :] = v[64:128]
        if zn is not None:
            t_ref[0, n2, 512:KR_, :] = k1[128:136]
            t_ref[1, n2, 512:KR_, :] = im[128:136]

    ye = butterflies(False)
    z0 = feature_stage(0, ye[0:2])
    z2 = feature_stage(2, ye[2:5])
    yo = butterflies(True)
    sequence_stage(0, *z0)
    z1 = feature_stage(1, yo[0:3])
    sequence_stage(2, *z2)
    z3 = feature_stage(3, yo[3:6])
    sequence_stage(1, *z1)
    sequence_stage(3, *z3)


def _inverse_rows(t_ref, dmat_ref, smat_ref, imat_ref, n2):
    def dm(i):
        return _bf(dmat_ref[i * 64:(i + 1) * 64, :])

    row = lax.broadcasted_iota(jnp.int32, (8, 128), 0)
    lane = lax.broadcasted_iota(jnp.int32, (1, 128), 1)
    sgn = jnp.where(lane < 64, 1.0, -1.0).astype(f32)
    mcd = jnp.concatenate([_bf(smat_ref[n2, 0]), _bf(imat_ref[4 + n2])], axis=1)
    vr, vi = t_ref[0, n2, 0:64, :], t_ref[1, n2, 0:64, :]
    nr, ni = t_ref[0, n2, 512:KR_, :], t_ref[1, n2, 512:KR_, :]
    vi0 = jnp.concatenate([jnp.where(row == 0, nr, vi[0:8]), vi[8:64]], axis=0)
    vr0 = jnp.concatenate([jnp.where(row == 0, ni, -vr[0:8]), -vr[8:64]], axis=0)
    ra = jnp.concatenate([jnp.concatenate([vr, vi0], axis=0),
                          jnp.concatenate([vi, vr0], axis=0)], axis=1).astype(bf16)
    ta = _dot_nt(mcd, ra)
    vr, vi = t_ref[0, n2, 256:320, :], t_ref[1, n2, 256:320, :]
    rb = jnp.concatenate([jnp.concatenate([vr, vi], axis=0),
                          jnp.concatenate([vi, -vr], axis=0)], axis=1).astype(bf16)
    tb = _dot_nt(mcd, rb)
    us = []
    for r in (1, 2, 3):
        vr, vi = [jnp.concatenate([t_ref[ri, n2, 64 * r:64 * r + 64, :],
                                   t_ref[ri, n2, 64 * (8 - r):64 * (9 - r), :]], axis=0) for ri in range(2)]
        k1 = _dot_nt(_bf(smat_ref[n2, 0]), (vr + vi).astype(bf16))
        k2 = _dot_nt(_bf(smat_ref[n2, 2]), vr.astype(bf16))
        k3 = _dot_nt(_bf(smat_ref[n2, 1]), vi.astype(bf16))
        us.append((k1 + k3, (k1 - k2) * sgn))
    g0 = _dot(ta, _bf(imat_ref[0]))
    g4 = _dot(tb, dm(0))
    hr, hi = [], []
    for r in (1, 2, 3):
        ur, ui = us[r - 1]
        k1 = _dot(ur + ui, dm(3 * r - 2))
        k2 = _dot(ur, dm(3 * r - 1))
        k3 = _dot(ui, _bf(imat_ref[r]))
        hr.append(k1 + k3)
        hi.append(k1 - k2)
    ep, em = g0 + g4, g0 - g4
    s13 = hr[0] + hr[2]
    d13 = hi[0] - hi[2]
    p = ((hr[0] - hi[0]) - (hr[2] + hi[2])) * R2
    q = ((hr[2] - hi[2]) - (hr[0] + hi[0])) * R2
    e1, e2 = ep + hr[1], ep - hr[1]
    e3, e4 = em - hi[1], em + hi[1]
    return [e1 + s13, e3 + p, e2 - d13, e4 + q, e1 - s13, e3 - p, e2 + d13, e4 - q]


def _filter_rows(t_ref, row0, get_w):
    rows = pl.ds(row0, 8)
    xf = _fft16([(t_ref[0, n2, rows, :], t_ref[1, n2, rows, :]) for n2 in range(16)], -1)
    prod = []
    for k2 in range(16):
        wr, wi = get_w(k2)
        xr, xi = xf[k2]
        prod.append((xr * wr - xi * wi, xr * wi + xi * wr))
    vs = _fft16(prod, +1)
    for n2 in range(16):
        t_ref[0, n2, rows, :] = vs[n2][0]
        t_ref[1, n2, rows, :] = vs[n2][1]


def _segment_schedule(order="ps2o10", lag_s=2, lag_p=2, lag_o=0, groups=(4, 4, 4, 4, 4, 4, 2, 2, 2, 2),
                      hold=5, spread=8, spread_tail=2):
    bounds = [sum(groups[:g]) for g in range(len(groups) + 1)]
    first_held = len(groups) - 1 - hold
    shares = {}
    for g in range(len(groups)):
        if g == len(groups) - 1:
            slot, parts, step = 10 ** 6, spread_tail, 0
        elif g >= first_held:
            slot, parts, step = H_ + (g - first_held) * (lag_s + lag_p) // hold, spread_tail, 1
        else:
            slot, step = bounds[g + 1] - 1 + lag_s + lag_p + lag_o, 1
            parts = spread if slot < H_ else spread_tail
        for k in range(parts):
            cols = tuple(range(k * 8 // parts, (k + 1) * 8 // parts))
            shares.setdefault(slot + k * step, []).append(("o", bounds[g], bounds[g + 1], cols))
    sched = []
    for i in range(H_ + lag_s + lag_p):
        for ch in order:
            if ch in "012" and i < H_:
                sched.append(("proj", i, int(ch)))
            elif ch == "o":
                sched += shares.pop(i, [])
            elif ch == "s" and 0 <= i - lag_s < H_:
                sched.append(("s", i - lag_s))
            elif ch == "p" and 0 <= i - lag_s - lag_p < H_:
                sched.append(("pv", i - lag_s - lag_p))
    for slot in sorted(shares):
        sched += shares[slot]
    return sched


def _kernel(ax_hbm, wrt_hbm, wit_hbm, dmat_hbm, smat_hbm, imat_hbm,
            bx_hbm, m0_hbm, wq_hbm, wk_hbm, wv_hbm, wo_hbm, out_hbm,
            xg_ref, t_ref, fw_ref, fn_ref, dmat_ref, smat_ref, imat_ref,
            w_ref, wo_ref, bxa_ref, bxp_ref, m0_ref, xp_ref, pre_ref, outb_ref,
            sem_ax, sem_c, sem_fw, sem_w, sem_late, sem_bx, sem_outa, sem_outb):
    axu = ax_hbm.bitcast(u32)
    outu = out_hbm.bitcast(u32)
    w_hbm = [w.bitcast(u32) for w in (wq_hbm, wk_hbm, wv_hbm)]
    wou = wo_hbm.bitcast(u32)

    def ax_copies(c):
        pair = pl.ds(2 * c, 2)
        return [pltpu.make_async_copy(axu.at[:, c], xg_ref.at[c], sem_ax.at[c]),
                pltpu.make_async_copy(smat_hbm.at[pair], smat_ref.at[pair], sem_c.at[1 + c])]

    def w_copies(j, mi):
        return [pltpu.make_async_copy(w_hbm[mi].at[:, par * 16 + j], w_ref.at[mi, 2 * j + par],
                                      sem_w.at[3 * j + mi]) for par in range(2)]

    def outa_copy(c):
        return pltpu.make_async_copy(xg_ref.at[c], outu.at[:, c, pl.ds(0, D_)], sem_outa.at[0])

    def outb_copy(s0, n):
        blk = pl.ds(2 * s0, 2 * n)
        return pltpu.make_async_copy(outb_ref.at[blk], out_hbm.at[blk, :, pl.ds(D_, D_)], sem_outb.at[0])

    dmat_copy = pltpu.make_async_copy(dmat_hbm, dmat_ref, sem_c.at[0])
    bxp_copy = pltpu.make_async_copy(bx_hbm.at[:, pl.ds(TOK_, PRE_)], bxp_ref, sem_bx.at[0])
    fwu = [wh.at[pl.ds(0, 512)].bitcast(u32) for wh in (wrt_hbm, wit_hbm)]

    def fw_copy(ri, k2):
        lanes = pl.ds(pl.multiple_of(k2 * 128, 128), 128)
        return pltpu.make_async_copy(fwu[ri].at[:, lanes], fw_ref.at[ri, k2, pl.ds(0, 256)], sem_fw.at[0])

    inv_copies = [pltpu.make_async_copy(wh.at[pl.ds(512, 1)], fn_ref.at[ri], sem_fw.at[1])
                  for ri, wh in enumerate((wrt_hbm, wit_hbm))]
    inv_copies.append(pltpu.make_async_copy(imat_hbm, imat_ref, sem_fw.at[1]))

    def wo_copy(n):
        lanes = pl.ds(pl.multiple_of(n * 128, 128), 128)
        return pltpu.make_async_copy(wou.at[:, lanes], wo_ref.at[n], sem_late.at[0])

    late_copies = [pltpu.make_async_copy(bx_hbm.at[:, pl.ds(0, TOK_)], bxa_ref, sem_late.at[1]),
                   pltpu.make_async_copy(m0_hbm, m0_ref, sem_late.at[1])]

    def start_pair(j):
        for mi in range(3):
            for cp in w_copies(j, mi):
                cp.start()

    for c in range(8):
        for cp in ax_copies(c):
            cp.start()
        if c == 0:
            dmat_copy.start()

    def forward(chunks):
        for c in chunks:
            for cp in ax_copies(c):
                cp.wait()
        for c in chunks:
            for par in range(2):
                _forward_rows(xg_ref, t_ref, dmat_ref, smat_ref, c, par)

    def forward_pair(i, carry):
        forward([2 * i + 1, 2 * i + 2])
        start_pair(i + 1)
        return carry

    dmat_copy.wait()
    forward([0])
    bxp_copy.start()
    start_pair(0)
    lax.fori_loop(0, 3, forward_pair, 0)
    forward([7])

    def relayout(j, mi):
        for r in range(0, 512, 64):
            a = w_ref[mi, 2 * j, r:r + 64, :]
            b = w_ref[mi, 2 * j + 1, r:r + 64, :]
            w_ref[mi, 2 * j, r:r + 64, :] = (a & LO16) | (b << 16)
            w_ref[mi, 2 * j + 1, r:r + 64, :] = (a >> 16) | (b & HI16)

    bxp_copy.wait()
    for i in range(0, NSEG_, 2):
        v = jnp.concatenate([bxp_ref[i].astype(f32), bxp_ref[i + 1].astype(f32)], axis=0)
        xp_ref[i * 4:i * 4 + 8, :] = pltpu.bitcast(v.astype(bf16), u32)
    for cp in w_copies(0, 0):
        cp.wait()
    relayout(0, 0)

    def early_rows(j, carry, last=False):
        todo = [(j, 1), (j, 2)]
        if last:
            todo += [(jj, mi) for jj in range(NPAIR_, H_ // 2) for mi in range(3)]
            for cp in late_copies:
                cp.start()
        else:
            todo += [(j + 1, 0)]
        for it in todo:
            for cp in w_copies(*it):
                cp.wait()
        for mi in range(3):
            xp = _bf(xp_ref[...])
            for hh in range(2):
                pre_ref[mi, 2 * j + hh] = _dot(xp, _bf(w_ref[mi, 2 * j + hh]))
            for it in todo[mi::3]:
                relayout(*it)
        if not last:
            pl.when(j + AHEAD_ < H_ // 2)(lambda: start_pair(j + AHEAD_))

            @pl.when(j < 8)
            def _():
                for ri in range(2):
                    for k in range(2):
                        fw_copy(ri, 2 * j + k).start()

            pl.when(j >= NPAIR_ - 9)(lambda: wo_copy(j - (NPAIR_ - 9)).start())
        return carry

    for cp in inv_copies:
        cp.start()
    lax.fori_loop(0, NPAIR_ - 1, early_rows, 0)
    early_rows(NPAIR_ - 1, 0, last=True)

    fw_all = fw_ref.at[:, :, pl.ds(0, 256)]
    pltpu.make_async_copy(fw_all, fw_all, sem_fw.at[0]).wait()
    for cp in inv_copies:
        cp.wait()

    def filter_pair(m):
        cls, g = m // 8, m % 8
        for odd in range(2):
            def get_w(k2):
                idx = pl.ds(g * 32 + cls, 8, stride=4)
                a, b = fw_ref[0, k2, idx, :], fw_ref[1, k2, idx, :]
                a, b = (a & HI16, b & HI16) if odd else (a << 16, b << 16)
                return pltpu.bitcast(a, f32), pltpu.bitcast(b, f32)

            _filter_rows(t_ref, pl.multiple_of((2 * cls + odd) * 64 + g * 8, 8), get_w)

    def filter_pairs(i, carry):
        for u in range(2):
            filter_pair(2 * i + u)
        return carry

    lax.fori_loop(0, 16, filter_pairs, 0)
    _filter_rows(t_ref, 512, lambda k2: tuple(
        jnp.broadcast_to(fn_ref[ri, :, k2 * 128:(k2 + 1) * 128].astype(f32), (8, 128)) for ri in range(2)))

    def inverse(i, carry):
        for u in range(4):
            c = 4 * i + u
            res = [_inverse_rows(t_ref, dmat_ref, smat_ref, imat_ref, 2 * c + par) for par in range(2)]
            for a in range(8):
                even, odd = [pltpu.bitcast(r[a].astype(bf16).astype(f32), u32) for r in res]
                xg_ref[c, :, a * 128:(a + 1) * 128] = (even >> 16) | (odd & HI16)
        for u in range(4):
            outa_copy(4 * i + u).start()
        return carry

    lax.fori_loop(0, 2, inverse, 0)

    pltpu.make_async_copy(wo_ref, wo_ref, sem_late.at[0]).wait()
    for cp in late_copies:
        cp.wait()
    sched = _segment_schedule()

    def head(t):
        return (t - NFULL_) % H_

    def segment(s, mem):
        early = pl.ds(pl.multiple_of(s * PRE_, PRE_), PRE_)
        row = lax.broadcasted_iota(jnp.int32, (L_, L_), 0)
        col = lax.broadcasted_iota(jnp.int32, (L_, L_), 1)
        mask = (row < M_) | (row >= col)
        xs = bxa_ref[s].astype(f32)
        h32 = jnp.concatenate(
            [jnp.concatenate([mem[n], xs[:, n * 128:(n + 1) * 128]], axis=0) for n in range(8)], axis=1)
        h40 = jnp.concatenate([h32, bxp_ref[s].astype(f32)], axis=0)
        proj, probs, att = {}, {}, {}
        acc = [None] * 8
        for op in sched:
            if op[0] == "proj":
                _, t, mi = op
                w = _bf(w_ref[mi, head(t)])
                if t < NFULL_:
                    y = _dot(h40, w)
                else:
                    y = jnp.concatenate([_dot(h32, w), pre_ref[mi, head(t), early, :]], axis=0)
                proj[t, mi] = y if mi == 0 else y.astype(bf16)
            elif op[0] == "s":
                t = op[1]
                qk = _dot_nt(proj.pop((t, 0)), proj.pop((t, 1)))
                sc = jnp.where(mask, qk * (DH_ ** -0.5 * LOG2E), -1e9 * LOG2E)
                e = jnp.exp2(sc - jnp.max(sc, axis=-1, keepdims=True))
                probs[t] = (e, pl.reciprocal(jnp.sum(e, axis=-1, keepdims=True)))
            elif op[0] == "pv":
                t = op[1]
                e, inv_sum = probs.pop(t)
                att[t] = _dot(e, proj.pop((t, 2))) * inv_sum
            else:
                _, t0, t1, cols = op
                og = jnp.concatenate([att[t] for t in range(t0, t1)], axis=1)
                for n in cols:
                    y = _dot(og, _bf(wo_ref[n, head(t0) * 64:(head(t1 - 1) + 1) * 64, :]))
                    acc[n] = y if acc[n] is None else acc[n] + y
        for n in range(8):
            yb = acc[n][M_:].astype(bf16)
            outb_ref[2 * s, :, n * 128:(n + 1) * 128] = yb[0:16]
            outb_ref[2 * s + 1, :, n * 128:(n + 1) * 128] = yb[16:32]
        return tuple(acc[n][0:M_] for n in range(8))

    def segments(i, mem):
        for u in range(UNROLL_):
            mem = segment(i * UNROLL_ + u, mem)
            if u == UNROLL_ - 2:
                outb_copy(i * UNROLL_, UNROLL_ - 1).start()
        outb_copy(i * UNROLL_ + UNROLL_ - 1, 1).start()
        return mem

    m0 = m0_ref[...].astype(f32)
    lax.fori_loop(0, NSEG_ // UNROLL_, segments, tuple(m0[:, n * 128:(n + 1) * 128] for n in range(8)))
    for c in range(8):
        outa_copy(c).wait()
    outb_copy(0, NSEG_).wait()


@functools.partial(jax.jit, static_argnames=("B_seg_len",))
def pallas_concat_heads__spectral_gfnet__memory_aug_recurrent_mem_tr__prompt_kernel(
    A_x: jax.Array,
    A_w_r: jax.Array,
    A_w_i: jax.Array,
    B_x: jax.Array,
    B_mem0: jax.Array,
    B_Wq: jax.Array,
    B_Wk: jax.Array,
    B_Wv: jax.Array,
    B_Wo: jax.Array,
    B_seg_len: int,
):
    assert B_seg_len == SEG_
    assert A_x.shape == (1, S_, D_) and B_x.shape == (1, S_, D_)
    assert B_Wq.shape == (D_, H_, DH_) and B_mem0.shape == (1, M_, D_)
    hbm = pl.BlockSpec(memory_space=pltpu.HBM)
    dma = pltpu.SemaphoreType.DMA
    out = pl.pallas_call(
        _kernel,
        out_shape=jax.ShapeDtypeStruct((128, 16, 2 * D_), bf16),
        in_specs=[hbm] * 12,
        out_specs=hbm,
        scratch_shapes=[
            pltpu.VMEM((8, 128, D_), u32),
            pltpu.VMEM((2, 16, KR_, 128), f32),
            pltpu.VMEM((2, 16, 264, 128), u32),
            pltpu.VMEM((2, 1, S_), bf16),
            pltpu.VMEM(_DMAT.shape, u32),
            pltpu.VMEM(_SMAT.shape, u32),
            pltpu.VMEM(_IMAT.shape, u32),
            pltpu.VMEM((3, H_, D_ // 2, DH_), u32),
            pltpu.VMEM((8, H_ * DH_ // 2, 128), u32),
            pltpu.VMEM((NSEG_, TOK_, D_), bf16),
            pltpu.VMEM((NSEG_, PRE_, D_), bf16),
            pltpu.VMEM((M_, D_), bf16),
            pltpu.VMEM((NSEG_ * PRE_ // 2, D_), u32),
            pltpu.VMEM((3, H_ - NFULL_, NSEG_ * PRE_, DH_), f32),
            pltpu.VMEM((128, 16, D_), bf16),
            dma((8,)), dma((9,)), dma((2,)), dma((3 * H_ // 2,)), dma((2,)), dma((1,)), dma((1,)), dma((1,)),
        ],
        compiler_params=pltpu.CompilerParams(
            vmem_limit_bytes=120 * 1024 * 1024,
            flags={"XLA_TPU_EVENLY_DISTRIBUTE_CRITICAL_NODES": True}),
    )(A_x.reshape(128, 16, D_), A_w_r.T, A_w_i.T, _DMAT, _SMAT, _IMAT,
      B_x.reshape(NSEG_, SEG_, D_), B_mem0.reshape(M_, D_),
      B_Wq.reshape(D_ // 2, 2 * H_, DH_), B_Wk.reshape(D_ // 2, 2 * H_, DH_), B_Wv.reshape(D_ // 2, 2 * H_, DH_),
      B_Wo.reshape(H_ * DH_, D_))
    return out.reshape(1, S_, 2 * D_)
```

```python
import functools

import jax
import jax.numpy as jnp
import ml_dtypes
import numpy as np
from jax import lax
import jax.experimental.pallas as pl
import jax.experimental.pallas.tpu as pltpu

S_, D_, H_, DH_, M_, SEG_ = 2048, 1024, 32, 128, 8, 32
L_ = M_ + SEG_
NSEG_ = S_ // SEG_
PRE_ = 8
TOK_ = SEG_ - PRE_
KR_ = 520
AHEAD_ = 4
NFULL_ = 4
NPAIR_ = (H_ - NFULL_) // 2
UNROLL_ = 4
f32, bf16, u32 = jnp.float32, jnp.bfloat16, jnp.uint32
HI16 = np.uint32(0xFFFF0000)
LO16 = np.uint32(0xFFFF)
R2 = float(np.sqrt(0.5))
LOG2E = float(np.log2(np.e))


def _dft_constants():
    th = 2 * np.pi / D_
    b = np.arange(128)
    j = np.arange(64)

    def cs(k):
        ang = th * ((k[:, None] * b[None, :]) % D_)
        return np.cos(ang), np.sin(ang)

    c0, s0 = cs(8 * j)
    c4, s4 = cs(4 + 8 * j)
    alt = (-1.0) ** b
    nyq = np.zeros((16, 128))
    nyq[0] = alt
    l0 = np.concatenate([c0, -s0], 0)
    l4 = np.concatenate([c4, -s4], 0)
    i0 = l0.copy()
    i0[0] *= 0.5
    i0[64] = 0.5 * alt
    fwd, inv = [l4], [i0]
    lower = np.where(np.arange(128) < 64, 1.0, -1.0)[:, None]
    for r in (1, 2, 3):
        ca, sa = cs(r + 8 * j)
        cb, sb = cs(8 - r + 8 * j)
        c = np.concatenate([ca, cb], 0)
        d = np.concatenate([-sa, sb], 0)
        fwd += [c, c + d, (d - c) * lower]
        inv += [d - c]
    n1 = np.arange(128)
    seq = []
    for n2 in range(16):
        ang = 2 * np.pi / S_ * (((16 * n1 + n2)[:, None] * n1[None, :]) % S_)
        c, d = np.cos(ang) * 2.0 ** -10, -np.sin(ang) * 2.0 ** -10
        seq.append(np.stack([c, d - c, c + d]))
        inv.append(d)

    def words(m):
        u = m.astype(ml_dtypes.bfloat16).view(np.uint16).astype(np.uint32)
        return u[..., 0::2, :] | (u[..., 1::2, :] << 16)

    return words(np.concatenate(fwd + [l0, nyq], 0)), words(np.stack(seq)), words(np.stack(inv))


_DMAT, _SMAT, _IMAT = _dft_constants()


def _bf(words):
    return pltpu.bitcast(words, bf16)


def _dot_nt(a, b):
    return lax.dot_general(a, b, (((1,), (1,)), ((), ())), preferred_element_type=f32)


def _dot(a, b):
    return jnp.dot(a, b, preferred_element_type=f32)


def _radix4(xs, sgn):
    (ar, ai), (br, bi), (cr, ci), (dr, di) = xs
    t0r, t0i = ar + cr, ai + ci
    t1r, t1i = ar - cr, ai - ci
    t2r, t2i = br + dr, bi + di
    t3r, t3i = br - dr, bi - di
    y0 = (t0r + t2r, t0i + t2i)
    y2 = (t0r - t2r, t0i - t2i)
    ym = (t1r + t3i, t1i - t3r)
    yp = (t1r - t3i, t1i + t3r)
    return [y0, ym, y2, yp] if sgn < 0 else [y0, yp, y2, ym]


def _twiddle16(z, e, sgn):
    r, i = z
    if e == 0:
        return z
    if e == 4:
        return (-i, r) if sgn > 0 else (i, -r)
    if e == 2:
        return ((r - i) * R2, (r + i) * R2) if sgn > 0 else ((r + i) * R2, (i - r) * R2)
    if e == 6:
        return ((-r - i) * R2, (r - i) * R2) if sgn > 0 else ((i - r) * R2, (-r - i) * R2)
    c = float(np.cos(2 * np.pi * e / 16))
    s = float(sgn * np.sin(2 * np.pi * e / 16))
    return (r * c - i * s, r * s + i * c)


def _fft16(xs, sgn):
    a = [_radix4([xs[4 * p + q] for p in range(4)], sgn) for q in range(4)]
    out = [None] * 16
    for u in range(4):
        y = _radix4([_twiddle16(a[q][u], q * u, sgn) for q in range(4)], sgn)
        for v in range(4):
            out[u + 4 * v] = y[v]
    return out


def _forward_rows(xg_ref, t_ref, dmat_ref, smat_ref, c, par):
    n2 = 2 * c + par

    def dm(i):
        return _bf(dmat_ref[i * 64:(i + 1) * 64, :])

    def butterflies(odd):
        outs = []
        for r0 in range(0, 128, 16):
            w = [xg_ref[c, r0:r0 + 16, a * 128:(a + 1) * 128] for a in range(8)]
            xa = [pltpu.bitcast((v << 16) if par == 0 else (v & HI16), f32) for v in w]
            if odd:
                t1, t3, t5, t7 = xa[0] - xa[4], xa[2] - xa[6], xa[1] - xa[5], xa[3] - xa[7]
                u, v = (t5 - t7) * R2, (t5 + t7) * -R2
                p1, q1, p3, q3 = t1 + u, v - t3, t1 - u, t3 + v
                ys = [p1, q1, p1 + q1, p3, q3, p3 + q3]
            else:
                t0, t2, t4, t6 = xa[0] + xa[4], xa[2] + xa[6], xa[1] + xa[5], xa[3] + xa[7]
                e, o = t0 + t2, t4 + t6
                p2, q2 = t0 - t2, t6 - t4
                ys = [e + o, e - o, p2, q2, p2 + q2]
            outs.append([yv.astype(bf16) for yv in ys])
        return [jnp.concatenate(col, axis=0) for col in zip(*outs)]

    def feature_stage(r, ys):
        if r == 0:
            z0 = _dot_nt(_bf(dmat_ref[10 * 64:10 * 64 + 72, :]), ys[0])
            z4 = _dot_nt(dm(0), ys[1])
            return (jnp.concatenate([z0[0:64], z4[0:64]], axis=0),
                    jnp.concatenate([z0[64:128], z4[64:128]], axis=0), z0[128:136])
        p, q, pq = ys
        k1 = _dot_nt(dm(3 * r - 2), pq)
        k2 = _dot_nt(dm(3 * r), p)
        k3 = _dot_nt(dm(3 * r - 1), q)
        return k1 - k3, jnp.concatenate([k1[0:64] + k2[0:64], k2[64:128] - k1[64:128]], axis=0), None

    def sequence_stage(r, zr, zi, zn):
        zs = zr + zi
        if zn is not None:
            zs, zr = jnp.concatenate([zs, zn], axis=0), jnp.concatenate([zr, zn], axis=0)
        k1 = _dot(zs, _bf(smat_ref[n2, 0]))
        k2 = _dot(zr, _bf(smat_ref[n2, 1]))
        k3 = _dot(zi, _bf(smat_ref[n2, 2]))
        re, im = k1[0:128] - k3, k1 + k2
        ra, rb = (0, 4) if r == 0 else (r, 8 - r)
        for ri, v in enumerate((re, im)):
            t_ref[ri, n2, 64 * ra:64 * ra + 64, :] = v[0:64]
            t_ref[ri, n2, 64 * rb:64 * rb + 64, :] = v[64:128]
        if zn is not None:
            t_ref[0, n2, 512:KR_, :] = k1[128:136]
            t_ref[1, n2, 512:KR_, :] = im[128:136]

    ye = butterflies(False)
    z0 = feature_stage(0, ye[0:2])
    z2 = feature_stage(2, ye[2:5])
    yo = butterflies(True)
    sequence_stage(0, *z0)
    z1 = feature_stage(1, yo[0:3])
    sequence_stage(2, *z2)
    z3 = feature_stage(3, yo[3:6])
    sequence_stage(1, *z1)
    sequence_stage(3, *z3)


def _inverse_rows(t_ref, dmat_ref, smat_ref, imat_ref, n2):
    def dm(i):
        return _bf(dmat_ref[i * 64:(i + 1) * 64, :])

    row = lax.broadcasted_iota(jnp.int32, (8, 128), 0)
    lane = lax.broadcasted_iota(jnp.int32, (1, 128), 1)
    sgn = jnp.where(lane < 64, 1.0, -1.0).astype(f32)
    mcd = jnp.concatenate([_bf(smat_ref[n2, 0]), _bf(imat_ref[4 + n2])], axis=1)
    vr, vi = t_ref[0, n2, 0:64, :], t_ref[1, n2, 0:64, :]
    nr, ni = t_ref[0, n2, 512:KR_, :], t_ref[1, n2, 512:KR_, :]
    vi0 = jnp.concatenate([jnp.where(row == 0, nr, vi[0:8]), vi[8:64]], axis=0)
    vr0 = jnp.concatenate([jnp.where(row == 0, ni, -vr[0:8]), -vr[8:64]], axis=0)
    ra = jnp.concatenate([jnp.concatenate([vr, vi0], axis=0),
                          jnp.concatenate([vi, vr0], axis=0)], axis=1).astype(bf16)
    ta = _dot_nt(mcd, ra)
    vr, vi = t_ref[0, n2, 256:320, :], t_ref[1, n2, 256:320, :]
    rb = jnp.concatenate([jnp.concatenate([vr, vi], axis=0),
                          jnp.concatenate([vi, -vr], axis=0)], axis=1).astype(bf16)
    tb = _dot_nt(mcd, rb)
    us = []
    for r in (1, 2, 3):
        vr, vi = [jnp.concatenate([t_ref[ri, n2, 64 * r:64 * r + 64, :],
                                   t_ref[ri, n2, 64 * (8 - r):64 * (9 - r), :]], axis=0) for ri in range(2)]
        k1 = _dot_nt(_bf(smat_ref[n2, 0]), (vr + vi).astype(bf16))
        k2 = _dot_nt(_bf(smat_ref[n2, 2]), vr.astype(bf16))
        k3 = _dot_nt(_bf(smat_ref[n2, 1]), vi.astype(bf16))
        us.append((k1 + k3, (k1 - k2) * sgn))
    g0 = _dot(ta, _bf(imat_ref[0]))
    g4 = _dot(tb, dm(0))
    hr, hi = [], []
    for r in (1, 2, 3):
        ur, ui = us[r - 1]
        k1 = _dot(ur + ui, dm(3 * r - 2))
        k2 = _dot(ur, dm(3 * r - 1))
        k3 = _dot(ui, _bf(imat_ref[r]))
        hr.append(k1 + k3)
        hi.append(k1 - k2)
    ep, em = g0 + g4, g0 - g4
    s13 = hr[0] + hr[2]
    d13 = hi[0] - hi[2]
    p = ((hr[0] - hi[0]) - (hr[2] + hi[2])) * R2
    q = ((hr[2] - hi[2]) - (hr[0] + hi[0])) * R2
    e1, e2 = ep + hr[1], ep - hr[1]
    e3, e4 = em - hi[1], em + hi[1]
    return [e1 + s13, e3 + p, e2 - d13, e4 + q, e1 - s13, e3 - p, e2 + d13, e4 - q]


def _filter_rows(t_ref, row0, get_w):
    rows = pl.ds(row0, 8)
    xf = _fft16([(t_ref[0, n2, rows, :], t_ref[1, n2, rows, :]) for n2 in range(16)], -1)
    prod = []
    for k2 in range(16):
        wr, wi = get_w(k2)
        xr, xi = xf[k2]
        prod.append((xr * wr - xi * wi, xr * wi + xi * wr))
    vs = _fft16(prod, +1)
    for n2 in range(16):
        t_ref[0, n2, rows, :] = vs[n2][0]
        t_ref[1, n2, rows, :] = vs[n2][1]


def _segment_schedule(order="1s02po", lag_s=2, lag_p=2, lag_o=1, groups=(2,) * 16,
                      hold=5, spread=2, spread_tail=1):
    bounds = [sum(groups[:g]) for g in range(len(groups) + 1)]
    first_held = len(groups) - 1 - hold
    shares = {}
    for g in range(len(groups)):
        if g == len(groups) - 1:
            slot, parts, step = 10 ** 6, spread_tail, 0
        elif g >= first_held:
            slot, parts, step = H_ + (g - first_held) * (lag_s + lag_p) // hold, spread_tail, 1
        else:
            slot, step = bounds[g + 1] - 1 + lag_s + lag_p + lag_o, 1
            parts = spread if slot < H_ else spread_tail
        for k in range(parts):
            cols = tuple(range(k * 8 // parts, (k + 1) * 8 // parts))
            shares.setdefault(slot + k * step, []).append(("o", bounds[g], bounds[g + 1], cols))
    sched = []
    for i in range(H_ + lag_s + lag_p):
        for ch in order:
            if ch in "012" and i < H_:
                sched.append(("proj", i, int(ch)))
            elif ch == "o":
                sched += shares.pop(i, [])
            elif ch == "s" and 0 <= i - lag_s < H_:
                sched.append(("s", i - lag_s))
            elif ch == "p" and 0 <= i - lag_s - lag_p < H_:
                sched.append(("pv", i - lag_s - lag_p))
    for slot in sorted(shares):
        sched += shares[slot]
    return sched


def _kernel(ax_hbm, wrt_hbm, wit_hbm, dmat_hbm, smat_hbm, imat_hbm,
            bx_hbm, m0_hbm, wq_hbm, wk_hbm, wv_hbm, wo_hbm, out_hbm,
            xg_ref, t_ref, fw_ref, fn_ref, dmat_ref, smat_ref, imat_ref,
            w_ref, wo_ref, bxa_ref, bxp_ref, m0_ref, xp_ref, pre_ref, outb_ref,
            sem_ax, sem_c, sem_fw, sem_w, sem_late, sem_bx, sem_outa, sem_outb):
    axu = ax_hbm.bitcast(u32)
    outu = out_hbm.bitcast(u32)
    w_hbm = [w.bitcast(u32) for w in (wq_hbm, wk_hbm, wv_hbm)]
    wou = wo_hbm.bitcast(u32)

    def ax_copies(c):
        pair = pl.ds(2 * c, 2)
        return [pltpu.make_async_copy(axu.at[:, c], xg_ref.at[c], sem_ax.at[c]),
                pltpu.make_async_copy(smat_hbm.at[pair], smat_ref.at[pair], sem_c.at[1 + c])]

    def w_copies(j, mi):
        return [pltpu.make_async_copy(w_hbm[mi].at[:, par * 16 + j], w_ref.at[mi, 2 * j + par],
                                      sem_w.at[3 * j + mi]) for par in range(2)]

    def outa_copy(c):
        return pltpu.make_async_copy(xg_ref.at[c], outu.at[:, c, pl.ds(0, D_)], sem_outa.at[0])

    def outb_copy(s0, n):
        blk = pl.ds(2 * s0, 2 * n)
        return pltpu.make_async_copy(outb_ref.at[blk], out_hbm.at[blk, :, pl.ds(D_, D_)], sem_outb.at[0])

    dmat_copy = pltpu.make_async_copy(dmat_hbm, dmat_ref, sem_c.at[0])
    bxp_copy = pltpu.make_async_copy(bx_hbm.at[:, pl.ds(TOK_, PRE_)], bxp_ref, sem_bx.at[0])
    fwu = [wh.at[pl.ds(0, 512)].bitcast(u32) for wh in (wrt_hbm, wit_hbm)]

    def fw_copy(ri, k2):
        lanes = pl.ds(pl.multiple_of(k2 * 128, 128), 128)
        return pltpu.make_async_copy(fwu[ri].at[:, lanes], fw_ref.at[ri, k2, pl.ds(0, 256)], sem_fw.at[0])

    inv_copies = [pltpu.make_async_copy(wh.at[pl.ds(512, 1)], fn_ref.at[ri], sem_fw.at[1])
                  for ri, wh in enumerate((wrt_hbm, wit_hbm))]
    inv_copies.append(pltpu.make_async_copy(imat_hbm, imat_ref, sem_fw.at[1]))

    def wo_copy(n):
        lanes = pl.ds(pl.multiple_of(n * 128, 128), 128)
        return pltpu.make_async_copy(wou.at[:, lanes], wo_ref.at[n], sem_late.at[0])

    late_copies = [pltpu.make_async_copy(bx_hbm.at[:, pl.ds(0, TOK_)], bxa_ref, sem_late.at[1]),
                   pltpu.make_async_copy(m0_hbm, m0_ref, sem_late.at[1])]

    def start_pair(j):
        for mi in range(3):
            for cp in w_copies(j, mi):
                cp.start()

    for c in range(8):
        for cp in ax_copies(c):
            cp.start()
        if c == 0:
            dmat_copy.start()

    def wait_rows(chunks):
        for c in chunks:
            for cp in ax_copies(c):
                cp.wait()

    def forward(chunks):
        for c in chunks:
            for par in range(2):
                _forward_rows(xg_ref, t_ref, dmat_ref, smat_ref, c, par)

    def forward_pair(i, carry):
        chunks = [2 * i + 1, 2 * i + 2]
        wait_rows(chunks)
        forward(chunks)
        start_pair(i + 1)
        return carry

    def relayout(j, mi):
        for r in range(0, 512, 64):
            a = w_ref[mi, 2 * j, r:r + 64, :]
            b = w_ref[mi, 2 * j + 1, r:r + 64, :]
            w_ref[mi, 2 * j, r:r + 64, :] = (a & LO16) | (b << 16)
            w_ref[mi, 2 * j + 1, r:r + 64, :] = (a >> 16) | (b & HI16)

    dmat_copy.wait()
    wait_rows([0])
    forward([0])
    bxp_copy.start()
    start_pair(0)
    lax.fori_loop(0, 3, forward_pair, 0)
    wait_rows([7])
    bxp_copy.wait()
    for cp in w_copies(0, 0):
        cp.wait()
    forward([7])

    for i in range(0, NSEG_, 2):
        v = jnp.concatenate([bxp_ref[i].astype(f32), bxp_ref[i + 1].astype(f32)], axis=0)
        xp_ref[i * 4:i * 4 + 8, :] = pltpu.bitcast(v.astype(bf16), u32)
    relayout(0, 0)

    def early_rows(j, carry, last=False):
        todo = [(j, 1), (j, 2)]
        if last:
            todo += [(jj, mi) for jj in range(NPAIR_, H_ // 2) for mi in range(3)]
            for cp in late_copies:
                cp.start()
            for cp in inv_copies:
                cp.wait()
        else:
            todo += [(j + 1, 0)]
        for it in todo:
            for cp in w_copies(*it):
                cp.wait()
        for mi in range(3):
            xp = _bf(xp_ref[...])
            for hh in range(2):
                pre_ref[mi, 2 * j + hh] = _dot(xp, _bf(w_ref[mi, 2 * j + hh]))
            for it in todo[mi::3]:
                relayout(*it)
        if not last:
            pl.when(j + AHEAD_ < H_ // 2)(lambda: start_pair(j + AHEAD_))

            @pl.when(j < 8)
            def _():
                for ri in range(2):
                    for k in range(2):
                        fw_copy(ri, 2 * j + k).start()

            pl.when(j >= NPAIR_ - 9)(lambda: wo_copy(j - (NPAIR_ - 9)).start())
        return carry

    for cp in inv_copies:
        cp.start()
    lax.fori_loop(0, NPAIR_ - 1, early_rows, 0)
    early_rows(NPAIR_ - 1, 0, last=True)
    _filter_rows(t_ref, 512, lambda k2: tuple(
        jnp.broadcast_to(fn_ref[ri, :, k2 * 128:(k2 + 1) * 128].astype(f32), (8, 128)) for ri in range(2)))

    fw_all = fw_ref.at[:, :, pl.ds(0, 256)]
    pltpu.make_async_copy(fw_all, fw_all, sem_fw.at[0]).wait()

    def filter_pair(m):
        cls, g = m // 8, m % 8
        for odd in range(2):
            def get_w(k2):
                idx = pl.ds(g * 32 + cls, 8, stride=4)
                a, b = fw_ref[0, k2, idx, :], fw_ref[1, k2, idx, :]
                a, b = (a & HI16, b & HI16) if odd else (a << 16, b << 16)
                return pltpu.bitcast(a, f32), pltpu.bitcast(b, f32)

            _filter_rows(t_ref, pl.multiple_of((2 * cls + odd) * 64 + g * 8, 8), get_w)

    def filter_pairs(i, carry):
        for u in range(2):
            filter_pair(2 * i + u)
        return carry

    lax.fori_loop(0, 16, filter_pairs, 0)

    def inverse(i, carry):
        for u in range(4):
            c = 4 * i + u
            res = [_inverse_rows(t_ref, dmat_ref, smat_ref, imat_ref, 2 * c + par) for par in range(2)]
            for a in range(8):
                even, odd = [pltpu.bitcast(r[a].astype(bf16).astype(f32), u32) for r in res]
                xg_ref[c, :, a * 128:(a + 1) * 128] = (even >> 16) | (odd & HI16)
        for u in range(4):
            outa_copy(4 * i + u).start()
        return carry

    lax.fori_loop(0, 2, inverse, 0)

    pltpu.make_async_copy(wo_ref, wo_ref, sem_late.at[0]).wait()
    for cp in late_copies:
        cp.wait()
    sched = _segment_schedule()

    def head(t):
        return (t - NFULL_) % H_

    def segment(s, mem):
        early = pl.ds(pl.multiple_of(s * PRE_, PRE_), PRE_)
        row = lax.broadcasted_iota(jnp.int32, (L_, L_), 0)
        col = lax.broadcasted_iota(jnp.int32, (L_, L_), 1)
        mask = (row < M_) | (row >= col)
        xs = bxa_ref[s].astype(f32)
        h32 = jnp.concatenate(
            [jnp.concatenate([mem[n], xs[:, n * 128:(n + 1) * 128]], axis=0) for n in range(8)], axis=1)
        h40 = jnp.concatenate([h32, bxp_ref[s].astype(f32)], axis=0)
        h32 = h32.astype(bf16)
        proj, probs, att = {}, {}, {}
        acc = [None] * 8
        for op in sched:
            if op[0] == "proj":
                _, t, mi = op
                w = _bf(w_ref[mi, head(t)])
                if t < NFULL_:
                    y = _dot(h40, w)
                else:
                    y = jnp.concatenate([_dot(h32, w), pre_ref[mi, head(t), early, :]], axis=0)
                proj[t, mi] = y if mi == 0 else y.astype(bf16)
            elif op[0] == "s":
                t = op[1]
                qk = _dot_nt(proj.pop((t, 0)), proj.pop((t, 1)))
                sc = jnp.where(mask, qk * (DH_ ** -0.5 * LOG2E), -1e9 * LOG2E)
                e = jnp.exp2(sc - jnp.max(sc, axis=-1, keepdims=True))
                probs[t] = (e, pl.reciprocal(jnp.sum(e, axis=-1, keepdims=True)))
            elif op[0] == "pv":
                t = op[1]
                e, inv_sum = probs.pop(t)
                att[t] = _dot(e, proj.pop((t, 2))) * inv_sum
            else:
                _, t0, t1, cols = op
                og = jnp.concatenate([att[t] for t in range(t0, t1)], axis=1)
                for n in cols:
                    y = _dot(og, _bf(wo_ref[n, head(t0) * 64:(head(t1 - 1) + 1) * 64, :]))
                    acc[n] = y if acc[n] is None else acc[n] + y
        for n in range(8):
            yb = acc[n][M_:].astype(bf16)
            outb_ref[2 * s, :, n * 128:(n + 1) * 128] = yb[0:16]
            outb_ref[2 * s + 1, :, n * 128:(n + 1) * 128] = yb[16:32]
        return tuple(acc[n][0:M_] for n in range(8))

    def segments(i, mem):
        for u in range(UNROLL_):
            mem = segment(i * UNROLL_ + u, mem)
            if u == UNROLL_ - 2:
                outb_copy(i * UNROLL_, UNROLL_ - 1).start()
        outb_copy(i * UNROLL_ + UNROLL_ - 1, 1).start()
        return mem

    m0 = m0_ref[...].astype(f32)
    lax.fori_loop(0, NSEG_ // UNROLL_, segments, tuple(m0[:, n * 128:(n + 1) * 128] for n in range(8)))
    for c in range(8):
        outa_copy(c).wait()
    outb_copy(0, NSEG_).wait()


@functools.partial(jax.jit, static_argnames=("B_seg_len",))
def pallas_concat_heads__spectral_gfnet__memory_aug_recurrent_mem_tr__prompt_kernel(
    A_x: jax.Array,
    A_w_r: jax.Array,
    A_w_i: jax.Array,
    B_x: jax.Array,
    B_mem0: jax.Array,
    B_Wq: jax.Array,
    B_Wk: jax.Array,
    B_Wv: jax.Array,
    B_Wo: jax.Array,
    B_seg_len: int,
):
    assert B_seg_len == SEG_
    assert A_x.shape == (1, S_, D_) and B_x.shape == (1, S_, D_)
    assert B_Wq.shape == (D_, H_, DH_) and B_mem0.shape == (1, M_, D_)
    hbm = pl.BlockSpec(memory_space=pltpu.HBM)
    dma = pltpu.SemaphoreType.DMA
    out = pl.pallas_call(
        _kernel,
        out_shape=jax.ShapeDtypeStruct((128, 16, 2 * D_), bf16),
        in_specs=[hbm] * 12,
        out_specs=hbm,
        scratch_shapes=[
            pltpu.VMEM((8, 128, D_), u32),
            pltpu.VMEM((2, 16, KR_, 128), f32),
            pltpu.VMEM((2, 16, 264, 128), u32),
            pltpu.VMEM((2, 1, S_), bf16),
            pltpu.VMEM(_DMAT.shape, u32),
            pltpu.VMEM(_SMAT.shape, u32),
            pltpu.VMEM(_IMAT.shape, u32),
            pltpu.VMEM((3, H_, D_ // 2, DH_), u32),
            pltpu.VMEM((8, H_ * DH_ // 2, 128), u32),
            pltpu.VMEM((NSEG_, TOK_, D_), bf16),
            pltpu.VMEM((NSEG_, PRE_, D_), bf16),
            pltpu.VMEM((M_, D_), bf16),
            pltpu.VMEM((NSEG_ * PRE_ // 2, D_), u32),
            pltpu.VMEM((3, H_ - NFULL_, NSEG_ * PRE_, DH_), f32),
            pltpu.VMEM((128, 16, D_), bf16),
            dma((8,)), dma((9,)), dma((2,)), dma((3 * H_ // 2,)), dma((2,)), dma((1,)), dma((1,)), dma((1,)),
        ],
        compiler_params=pltpu.CompilerParams(
            vmem_limit_bytes=120 * 1024 * 1024,
            flags={"XLA_TPU_EVENLY_DISTRIBUTE_CRITICAL_NODES": True}),
    )(A_x.reshape(128, 16, D_), A_w_r.T, A_w_i.T, _DMAT, _SMAT, _IMAT,
      B_x.reshape(NSEG_, SEG_, D_), B_mem0.reshape(M_, D_),
      B_Wq.reshape(D_ // 2, 2 * H_, DH_), B_Wk.reshape(D_ // 2, 2 * H_, DH_), B_Wv.reshape(D_ // 2, 2 * H_, DH_),
      B_Wo.reshape(H_ * DH_, D_))
    return out.reshape(1, S_, 2 * D_)
```
